```python
import os as _os
_os.environ.setdefault("JAX_PLATFORMS", "cpu")
import jax
import jax.numpy as jnp

def _softmax(x, axis=-1):
    return jax.nn.softmax(x, axis=axis)
def _gelu(x):
    return jax.nn.gelu(x, approximate=True)
def _silu(x):
    return jax.nn.silu(x)
def _sigmoid(x):
    return jax.nn.sigmoid(x)
def _layernorm(x, axis=-1, eps=1e-5):
    m = jnp.mean(x, axis=axis, keepdims=True)
    v = jnp.var(x, axis=axis, keepdims=True)
    return (x - m) / jnp.sqrt(v + eps)
def _scatter_add(tgt, idx, src, axis=0):
    return tgt.at[idx].add(src)
def _segment_sum(src, seg, n):
    return jax.ops.segment_sum(src, seg, n)
class _Rng:
    def __init__(self, key):
        self._k = key
    def _next(self):
        self._k, sub = jax.random.split(self._k)
        return sub
    def normal(self, shape):
        return jax.random.normal(self._next(), shape, dtype=jnp.bfloat16)
    def randint(self, lo, hi, shape):
        return jax.random.randint(self._next(), shape, lo, hi, dtype=jnp.int32)
    def uniform(self, shape, lo=0.0, hi=1.0):
        return jax.random.uniform(self._next(), shape, jnp.bfloat16, lo, hi)
    def permutation(self, n):
        return jax.random.permutation(self._next(), n)


kernel_name = 'gated_mix__compressed_kv_cla__linear_attn_block__prompt'

def setup_inputs():
    _rng = _Rng(jax.random.key(int.from_bytes(__import__("os").urandom(4), "little")))
    _w = (lambda a: (lambda t: t.astype(jnp.bfloat16) if jnp.issubdtype(t.dtype, jnp.floating) else t)(jnp.asarray(a)))
    def _A_setup():
        B, H, Sq, Sk, D, M = 1, 16, 2048, 2048, 256, 448
        Dc = 4 * D
        return {
            "x": _w((lambda *s: _rng.normal(s) * 0.05)(B, Sq, M)),
            "c_kv": _w((lambda *s: _rng.normal(s) * 0.8)(B, Sk, Dc)),
            "w_q": _w((lambda *s: _rng.normal(s) * 3.2)(M, H, D) * (M ** -0.5)),
            "w_uk": _w((lambda *s: _rng.normal(s) * 3.2)(Dc, H, D) * (Dc ** -0.5)),
            "w_uv": _w((lambda *s: _rng.normal(s) * 0.8)(Dc, H, D) * (Dc ** -0.5)),
            "w_o": _w((lambda *s: _rng.normal(s) * 0.8)(H, D, M) * ((H * D) ** -0.5)),
        }
    _A_in = _A_setup()

    def _B_setup():
        B, S, D = 1, 2048, 448
        return {
            "x": _w((lambda *s: _rng.normal(s) * 0.05)(B, S, D)),
            "wqkv": _w((lambda *s: _rng.normal(s) * 1.6)(D, 3 * D)),
            "wo": _w((lambda *s: _rng.normal(s) * 0.4)(D, D)),
        }
    _B_in = _B_setup()

    return {
        "A_x": _A_in["x"],
        "A_c_kv": _A_in["c_kv"],
        "A_w_q": _A_in["w_q"],
        "A_w_uk": _A_in["w_uk"],
        "A_w_uv": _A_in["w_uv"],
        "A_w_o": _A_in["w_o"],
        "B_x": _B_in["x"],
        "B_wqkv": _B_in["wqkv"],
        "B_wo": _B_in["wo"],
        "gate_w": _w((lambda *s: _rng.normal(s) * 0.05)(448) * 16.0),
    }

def reference(A_x, A_c_kv, A_w_q, A_w_uk, A_w_uv, A_w_o, B_x, B_wqkv, B_wo, gate_w):
    def _A_ref(x, c_kv, w_q, w_uk, w_uv, w_o):
        B, Sq, M = x.shape[0], x.shape[1], x.shape[2]
        Sk = c_kv.shape[1]
        H, D = w_q.shape[1], w_q.shape[2]
        q = jnp.einsum("bqm,mhd->bhqd", x, w_q)
        k = jnp.einsum("bkc,chd->bhkd", c_kv, w_uk)
        v = jnp.einsum("bkc,chd->bhkd", c_kv, w_uv)
        scores = jnp.einsum("bhqd,bhkd->bhqk", q, k) * (D ** -0.5)
        off = Sk - Sq
        qi = jnp.arange(Sq)[:, None]
        kj = jnp.arange(Sk)[None, :]
        cmask = kj <= (qi + off)
        scores = jnp.where(cmask[None, None], scores, -1e9)
        p = _softmax(scores, axis=-1)
        ctx = jnp.einsum("bhqk,bhkd->bhqd", p, v)
        return jnp.einsum("bhqd,hdm->bqm", ctx, w_o)

    def _B_ref(x, wqkv, wo):
        B, S, D = x.shape
        H = 16; Dh = D // H
        qkv = (lambda x, *d: x.transpose(*d))((x @ wqkv).reshape(B, S, 3, H, Dh), 2, 0, 3, 1, 4)
        q, k, v = qkv[0], qkv[1], qkv[2]
        phi = lambda t: jnp.where(t > 0, t + 1, jnp.exp(t)) + 1e-6
        pq, pk = phi(q), phi(k)
        kv = jnp.einsum("bhsd,bhse->bhde", pk, v)
        z = jnp.einsum("bhsd->bhd", pk)
        num = jnp.einsum("bhqd,bhde->bhqe", pq, kv)
        den = jnp.einsum("bhqd,bhd->bhq", pq, z)[..., None] + 1e-6
        o = num / den
        return (lambda x, *d: x.transpose(*d))(o, 0, 2, 1, 3).reshape(B, S, D) @ wo

    x = A_x
    g = _sigmoid((x * gate_w).sum(-1, keepdims=True))
    a = _A_ref(x, A_c_kv, A_w_q, A_w_uk, A_w_uv, A_w_o)
    b = _B_ref(x, B_wqkv, B_wo)
    return g * a + (1 - g) * b
```

```python
import functools

import jax
import jax.numpy as jnp
import jax.experimental.pallas as pl
import jax.experimental.pallas.tpu as pltpu

_F32 = jnp.float32
_BF16 = jnp.bfloat16


def _nt(a, b):
    return jax.lax.dot_general(a, b, (((1,), (1,)), ((), ())), preferred_element_type=_F32)


def _tn(a, b):
    return jax.lax.dot_general(a, b, (((0,), (0,)), ((), ())), preferred_element_type=_F32)


def _nn(a, b):
    return jnp.dot(a, b, preferred_element_type=_F32)


def _kernel(x_ref, c_ref, wq_ref, wuk_ref, wuv_ref, wo_ref, wqkv_ref, wob_ref, gw_ref,
            o_ref, acc_ref, q_ref, k_ref, v_ref, ctx_ref, *, S, M, D, H, HB, TQ, scale):
    h = pl.program_id(0)
    nh = pl.num_programs(0)

    k_ref[...] = _nn(c_ref[...], wuk_ref[...]).astype(_BF16)
    v_ref[...] = _nn(c_ref[...], wuv_ref[...]).astype(_BF16)
    q_ref[...] = (_nn(x_ref[...], wq_ref[...]) * scale).astype(_BF16)

    row = jax.lax.broadcasted_iota(jnp.int32, (TQ, TQ), 0)
    col = jax.lax.broadcasted_iota(jnp.int32, (TQ, TQ), 1)
    cmask = col <= row
    for i in range(S // TQ):
        kv = (i + 1) * TQ
        qi = q_ref[i * TQ:(i + 1) * TQ, :]
        s = _nt(qi, k_ref[0:kv, :])
        sd = jnp.where(cmask, s[:, i * TQ:], -1e9)
        m = jnp.max(sd, axis=1, keepdims=True)
        if i > 0:
            so = s[:, :i * TQ]
            m = jnp.maximum(m, jnp.max(so, axis=1, keepdims=True))
            po = jnp.exp(so - m)
            pd = jnp.exp(sd - m)
            l = jnp.sum(po, axis=1, keepdims=True) + jnp.sum(pd, axis=1, keepdims=True)
            p = jnp.concatenate([po.astype(_BF16), pd.astype(_BF16)], axis=1)
        else:
            pd = jnp.exp(sd - m)
            l = jnp.sum(pd, axis=1, keepdims=True)
            p = pd.astype(_BF16)
        ctx = _nn(p, v_ref[0:kv, :]) / l
        ctx_ref[i * TQ:(i + 1) * TQ, :] = ctx.astype(_BF16)

    contrib = _nn(ctx_ref[...], wo_ref[...])

    @pl.when(h == 0)
    def _():
        acc_ref[...] = contrib

    @pl.when(h > 0)
    def _():
        acc_ref[...] += contrib

    @pl.when(h == nh - 1)
    def _():
        x = x_ref[...]
        Dh = M // HB
        qb = _nn(x, wqkv_ref[:, 0:M])
        kb = _nn(x, wqkv_ref[:, M:2 * M])
        vb = _nn(x, wqkv_ref[:, 2 * M:3 * M])
        phi = lambda t: jnp.where(t > 0, t + 1.0, jnp.exp(t)) + 1e-6
        pq = phi(qb)
        pk = phi(kb)
        kvm = _tn(pk.astype(_BF16), vb.astype(_BF16))
        z = jnp.sum(pk, axis=0, keepdims=True)
        hr = jax.lax.broadcasted_iota(jnp.int32, (M, M), 0) // Dh
        hc = jax.lax.broadcasted_iota(jnp.int32, (M, M), 1) // Dh
        same = hr == hc
        kvm = jnp.where(same, kvm, 0.0).astype(_BF16)
        ones_bd = jnp.where(same, 1.0, 0.0).astype(_BF16)
        num = _nn(pq.astype(_BF16), kvm)
        den = _nn((pq * z).astype(_BF16), ones_bd) + 1e-6
        ob = (num / den).astype(_BF16)
        b = _nn(ob, wob_ref[...])
        xf = x.astype(_F32)
        g = jax.nn.sigmoid(jnp.sum(xf * gw_ref[...].astype(_F32), axis=1, keepdims=True))
        o_ref[...] = (g * acc_ref[...] + (1.0 - g) * b).astype(o_ref.dtype)


@jax.jit
def pallas_gated_mix__compressed_kv_cla__linear_attn_block__prompt_kernel(
    A_x: jax.Array,
    A_c_kv: jax.Array,
    A_w_q: jax.Array,
    A_w_uk: jax.Array,
    A_w_uv: jax.Array,
    A_w_o: jax.Array,
    B_x: jax.Array,
    B_wqkv: jax.Array,
    B_wo: jax.Array,
    gate_w: jax.Array,
):
    B, S, M = A_x.shape
    Sk, Dc = A_c_kv.shape[1], A_c_kv.shape[2]
    H, D = A_w_q.shape[1], A_w_q.shape[2]
    assert B == 1 and S == Sk
    HB = 16
    TQ = 128

    x = A_x.reshape(S, M)
    c = A_c_kv.reshape(Sk, Dc)
    wq = A_w_q.reshape(M, H * D)
    wuk = A_w_uk.reshape(Dc, H * D)
    wuv = A_w_uv.reshape(Dc, H * D)
    wo = A_w_o.reshape(H * D, M)
    gw = gate_w.reshape(1, M)

    kern = functools.partial(_kernel, S=S, M=M, D=D, H=H, HB=HB, TQ=TQ, scale=float(D) ** -0.5)
    out = pl.pallas_call(
        kern,
        grid=(H,),
        in_specs=[
            pl.BlockSpec((S, M), lambda h: (0, 0)),
            pl.BlockSpec((Sk, Dc), lambda h: (0, 0)),
            pl.BlockSpec((M, D), lambda h: (0, h)),
            pl.BlockSpec((Dc, D), lambda h: (0, h)),
            pl.BlockSpec((Dc, D), lambda h: (0, h)),
            pl.BlockSpec((D, M), lambda h: (h, 0)),
            pl.BlockSpec((M, 3 * M), lambda h: (0, 0)),
            pl.BlockSpec((M, M), lambda h: (0, 0)),
            pl.BlockSpec((1, M), lambda h: (0, 0)),
        ],
        out_specs=pl.BlockSpec((S, M), lambda h: (0, 0)),
        out_shape=jax.ShapeDtypeStruct((S, M), A_x.dtype),
        scratch_shapes=[
            pltpu.VMEM((S, M), _F32),
            pltpu.VMEM((S, D), _BF16),
            pltpu.VMEM((Sk, D), _BF16),
            pltpu.VMEM((Sk, D), _BF16),
            pltpu.VMEM((S, D), _BF16),
        ],
        compiler_params=pltpu.CompilerParams(
            dimension_semantics=("arbitrary",),
            vmem_limit_bytes=100 * 1024 * 1024,
        ),
    )(x, c, wq, wuk, wuv, wo, B_wqkv, B_wo, gw)
    return out.reshape(B, S, M)
```

```python
import functools

import jax
import jax.numpy as jnp
import jax.experimental.pallas as pl
import jax.experimental.pallas.tpu as pltpu

_F32 = jnp.float32
_BF16 = jnp.bfloat16
def _nt(a, b): return jax.lax.dot_general(a, b, (((1,), (1,)), ((), ())), preferred_element_type=_F32)
def _nn(a, b): return jnp.dot(a, b, preferred_element_type=_F32)

def _kernel(xt_ref, wqkv_ref, wob_ref, gw_ref, c_hbm, wq_hbm, wuk_hbm, wuv_hbm, wot_hbm,
            o_ref,
            acc_ref, g_ref, c_ref, wot_ref, rq0, rq1, rk0, rk1, rv0, rv1, wqt_s, wk_s, wvt_s,
            qt_ref, k_ref, vt_ref, ctx_ref, wqkvt_ref, wobt_ref, pq_ref, kvt_ref, lhs_ref, e_ref, sems,
            *, S, M, D, Dc, H, HB, TQ, scale, variant, CP, CB, CO):
    h = pl.program_id(0)
    nh = pl.num_programs(0)
    L = 128
    HP = H // 2

    @pl.when(h == 0)
    def _():
        first = [
            pltpu.make_async_copy(wuv_hbm.at[:, 0:L], rv0, sems.at[4]),
            pltpu.make_async_copy(wuv_hbm.at[:, L:2 * L], rv1, sems.at[5]),
            pltpu.make_async_copy(wuk_hbm.at[:, 0:L], rk0, sems.at[2]),
            pltpu.make_async_copy(wuk_hbm.at[:, L:2 * L], rk1, sems.at[3]),
        ]
        second = [
            pltpu.make_async_copy(wq_hbm.at[:, 0:L], rq0, sems.at[0]),
            pltpu.make_async_copy(wq_hbm.at[:, L:2 * L], rq1, sems.at[1]),
            pltpu.make_async_copy(c_hbm, c_ref, sems.at[6]),
            pltpu.make_async_copy(wot_hbm, wot_ref, sems.at[7]),
        ]
        for cp in first:
            cp.start()
        if 'alldma' in variant:
            for cp in second:
                cp.start()

        Dh = M // HB
        wqkvt_ref[0:3 * M, :] = wqkv_ref[...].T
        wqkvt_ref[3 * M:3 * M + 16, :] = jnp.broadcast_to(gw_ref[...], (16, M))
        wobt_ref[...] = wob_ref[...].T
        kvt_ref[...] = jnp.zeros_like(kvt_ref)

        def b1(r, carry):
            cs = pl.ds(pl.multiple_of(r * CB, CB), CB)
            qkvt = _nn(wqkvt_ref[...], xt_ref[:, cs])
            g_ref[:, cs] = jax.nn.sigmoid(qkvt[3 * M:3 * M + 1, :])
            qk = qkvt[0:2 * M, :]
            pqk = (jnp.where(qk > 0, qk + 1.0, jnp.exp(qk)) + 1e-6).astype(_BF16)
            pq_ref[:, cs] = pqk[0:M, :]
            v_ext = jnp.concatenate([qkvt[2 * M:3 * M, :].astype(_BF16), jnp.ones((16, CB), _BF16)], axis=0)
            kvt_ref[...] += _nt(v_ext, pqk[M:2 * M, :])
            return carry
        jax.lax.fori_loop(0, S // CB, b1, 0)

        hr = jax.lax.broadcasted_iota(jnp.int32, (M, M), 0) // Dh
        hc = jax.lax.broadcasted_iota(jnp.int32, (M, M), 1) // Dh
        lhs_ref[0:M, :] = jnp.where(hr == hc, kvt_ref[0:M, :], 0.0).astype(_BF16)
        zr = jax.lax.broadcasted_iota(jnp.int32, (HB, M), 0)
        zc = jax.lax.broadcasted_iota(jnp.int32, (HB, M), 1) // Dh
        lhs_ref[M:M + HB, :] = jnp.where(zr == zc, kvt_ref[M:M + HB, :], 0.0).astype(_BF16)
        er = jax.lax.broadcasted_iota(jnp.int32, (M, 3 * HB), 0) // Dh
        ec = jax.lax.broadcasted_iota(jnp.int32, (M, 3 * HB), 1) % HB
        e_ref[...] = jnp.where(er == ec, 1.0, 0.0).astype(_BF16)

        for cp in first:
            cp.wait()
        if 'alldma' not in variant:
            for cp in second:
                cp.start()

        def split(raw, r, i, n):
            view = raw.bitcast(jnp.uint32).at[pl.ds(pl.multiple_of(r * (n * HP), n * HP), n * HP), :]
            u = view[pl.ds(i, n, stride=HP), :]
            lo = pltpu.bitcast(u << 16, _F32)
            hi = pltpu.bitcast(u & jnp.uint32(0xFFFF0000), _F32)
            return lo, hi

        def ext_kv(r):
            rs = pl.ds(pl.multiple_of(r * L, L), L)
            for i in range(HP):
                for j, (rk, rv) in enumerate(((rk0, rv0), (rk1, rv1))):
                    lo, hi = split(rk, r, i, L)
                    wk_s[2 * i, rs, j * L:(j + 1) * L] = lo.astype(_BF16)
                    wk_s[2 * i + 1, rs, j * L:(j + 1) * L] = hi.astype(_BF16)
                    lo, hi = split(rv, r, i, L)
                    wvt_s[2 * i, j * L:(j + 1) * L, rs] = lo.T.astype(_BF16)
                    wvt_s[2 * i + 1, j * L:(j + 1) * L, rs] = hi.T.astype(_BF16)

        nb = S // CB
        epb = (Dc // L) // nb
        def b2(r, carry):
            cs = pl.ds(pl.multiple_of(r * CB, CB), CB)
            nd = _nn(lhs_ref[...], pq_ref[:, cs])
            rc = 1.0 / (nd[M:M + HB, :] + 1e-6)
            r1 = rc.astype(_BF16)
            e1 = rc - r1.astype(_F32)
            r2 = e1.astype(_BF16)
            r3 = (e1 - r2.astype(_F32)).astype(_BF16)
            rx = _nn(e_ref[...], jnp.concatenate([r1, r2, r3], axis=0))
            ob = (nd[0:M, :] * rx).astype(_BF16)
            bt = _nn(wobt_ref[...], ob)
            acc_ref[:, cs] = (1.0 - g_ref[:, cs]) * bt
            for e in range(epb):
                ext_kv(r * epb + e)
            return carry
        jax.lax.fori_loop(0, nb, b2, 0)

        for cp in second:
            cp.wait()
        for i in range(HP):
            for j, rq in enumerate((rq0, rq1)):
                lo, hi = split(rq, 0, i, M)
                wqt_s[2 * i, j * L:(j + 1) * L, :] = (lo * scale).T.astype(_BF16)
                wqt_s[2 * i + 1, j * L:(j + 1) * L, :] = (hi * scale).T.astype(_BF16)

    def pbody(r, carry):
        rs = pl.ds(pl.multiple_of(r * CP, CP), CP)
        k_ref[rs, :] = _nn(c_ref[rs, :], wk_s[h]).astype(_BF16)
        vt_ref[:, rs] = _nt(wvt_s[h], c_ref[rs, :]).astype(_BF16)
        qt_ref[:, rs] = _nn(wqt_s[h], xt_ref[:, rs]).astype(_BF16)
        return carry
    jax.lax.fori_loop(0, S // CP, pbody, 0)

    row = jax.lax.broadcasted_iota(jnp.int32, (TQ, TQ), 0)
    col = jax.lax.broadcasted_iota(jnp.int32, (TQ, TQ), 1)
    cmask = row <= col
    nq = S // TQ
    def scores(i):
        kv = (i + 1) * TQ
        s = _nn(k_ref[0:kv, :], qt_ref[:, i * TQ:(i + 1) * TQ])
        sd = jnp.where(cmask, s[i * TQ:, :], -1e9)
        return (s[:i * TQ, :] if i > 0 else None), sd
    def smax(so, sd):
        m = jnp.max(sd, axis=0, keepdims=True)
        if so is not None:
            m = jnp.maximum(m, jnp.max(so, axis=0, keepdims=True))
        return m
    def sexp(so, sd, m):
        pd = jnp.exp(sd - m)
        l = jnp.sum(pd, axis=0, keepdims=True)
        if so is not None:
            po = jnp.exp(so - m)
            l = l + jnp.sum(po, axis=0, keepdims=True)
            p = jnp.concatenate([po.astype(_BF16), pd.astype(_BF16)], axis=0)
        else:
            p = pd.astype(_BF16)
        return p, l
    def pv(i, p, l):
        kv = (i + 1) * TQ
        r = g_ref[:, i * TQ:(i + 1) * TQ] / l
        ctx = _nn(vt_ref[:, 0:kv], p) * r
        ctx_ref[:, i * TQ:(i + 1) * TQ] = ctx.astype(_BF16)

    if 'noattn' not in variant:
        ss = [scores(j) for j in range(nq)]
        m = smax(*ss[0])
        for i in range(nq):
            p, l = sexp(*ss[i], m)
            if i + 1 < nq:
                m = smax(*ss[i + 1])
            pv(i, p, l)

    def obody(r, carry):
        cs = pl.ds(pl.multiple_of(r * CO, CO), CO)
        acc_ref[:, cs] += _nn(wot_ref[h], ctx_ref[:, cs])
        return carry
    jax.lax.fori_loop(0, S // CO, obody, 0)

    @pl.when(h == nh - 1)
    def _():
        o_ref[...] = acc_ref[...].astype(o_ref.dtype)

def build(TQ, variant, CP=512, CB=512, CO=1024):
    @jax.jit
    def f(A_x, A_c_kv, A_w_q, A_w_uk, A_w_uv, A_w_o, B_x, B_wqkv, B_wo, gate_w):
        B, S, M = A_x.shape
        Sk, Dc = A_c_kv.shape[1], A_c_kv.shape[2]
        H, D = A_w_q.shape[1], A_w_q.shape[2]
        HB = 16
        xt = A_x.reshape(S, M).T; c = A_c_kv.reshape(Sk, Dc)
        wq = A_w_q.reshape(M * H, D); wuk = A_w_uk.reshape(Dc * H, D); wuv = A_w_uv.reshape(Dc * H, D)
        wot = jnp.swapaxes(A_w_o, 1, 2); gw = gate_w.reshape(1, M)
        kern = functools.partial(_kernel, S=S, M=M, D=D, Dc=Dc, H=H, HB=HB, TQ=TQ, scale=float(D) ** -0.5, variant=variant, CP=CP, CB=CB, CO=CO)
        anyspec = pl.BlockSpec(memory_space=pl.ANY)
        out = pl.pallas_call(
            kern, grid=(H,),
            in_specs=[
                pl.BlockSpec((M, S), lambda h: (0, 0)),
                pl.BlockSpec((M, 3 * M), lambda h: (0, 0)),
                pl.BlockSpec((M, M), lambda h: (0, 0)),
                pl.BlockSpec((1, M), lambda h: (0, 0)),
                anyspec, anyspec, anyspec, anyspec, anyspec,
            ],
            out_specs=pl.BlockSpec((M, S), lambda h: (0, 0)),
            out_shape=jax.ShapeDtypeStruct((M, S), xt.dtype),
            scratch_shapes=[
                pltpu.VMEM((M, S), _F32), pltpu.VMEM((1, S), _F32),
                pltpu.VMEM((Sk, Dc), _BF16), pltpu.VMEM((H, M, D), _BF16),
                pltpu.VMEM((M * H, 128), _BF16), pltpu.VMEM((M * H, 128), _BF16),
                pltpu.VMEM((Dc * H, 128), _BF16), pltpu.VMEM((Dc * H, 128), _BF16),
                pltpu.VMEM((Dc * H, 128), _BF16), pltpu.VMEM((Dc * H, 128), _BF16),
                pltpu.VMEM((H, D, M), _BF16), pltpu.VMEM((H, Dc, D), _BF16), pltpu.VMEM((H, D, Dc), _BF16),
                pltpu.VMEM((D, S), _BF16), pltpu.VMEM((Sk, D), _BF16), pltpu.VMEM((D, Sk), _BF16), pltpu.VMEM((D, S), _BF16),
                pltpu.VMEM((3 * M + 16, M), _BF16), pltpu.VMEM((M, M), _BF16), pltpu.VMEM((M, S), _BF16),
                pltpu.VMEM((M + 16, M), _F32), pltpu.VMEM((M + HB, M), _BF16), pltpu.VMEM((M, 3 * HB), _BF16),
                pltpu.SemaphoreType.DMA((8,)),
            ],
            compiler_params=pltpu.CompilerParams(dimension_semantics=("arbitrary",), vmem_limit_bytes=110 * 1024 * 1024),
        )(xt, B_wqkv, B_wo, gw, c, wq, wuk, wuv, wot)
        return out.T.reshape(B, S, M)
    return f


_impl = build(128, (), CP=2048, CB=512, CO=2048)


@jax.jit
def pallas_gated_mix__compressed_kv_cla__linear_attn_block__prompt_kernel(
    A_x: jax.Array,
    A_c_kv: jax.Array,
    A_w_q: jax.Array,
    A_w_uk: jax.Array,
    A_w_uv: jax.Array,
    A_w_o: jax.Array,
    B_x: jax.Array,
    B_wqkv: jax.Array,
    B_wo: jax.Array,
    gate_w: jax.Array,
):
    return _impl(A_x, A_c_kv, A_w_q, A_w_uk, A_w_uv, A_w_o, B_x, B_wqkv, B_wo, gate_w)
```

```python
import functools

import jax
import jax.numpy as jnp
import jax.experimental.pallas as pl
import jax.experimental.pallas.tpu as pltpu

_F32 = jnp.float32
_BF16 = jnp.bfloat16
def _nt(a, b): return jax.lax.dot_general(a, b, (((1,), (1,)), ((), ())), preferred_element_type=_F32)
def _tn(a, b): return jax.lax.dot_general(a, b, (((0,), (0,)), ((), ())), preferred_element_type=_F32)
def _nn(a, b): return jnp.dot(a, b, preferred_element_type=_F32)

def _kernel(xt_hbm, wqkv_hbm, wob_hbm, gw_hbm, wot_hbm, c_hbm, wq_hbm, wuk_hbm, wuv_hbm,
            o_ref,
            xt_ref, wqkv_ref, wob_ref, gw_ref, xsems, acc_ref, g_ref, c_ref, wot_ref, rq0, rq1, rk0, rk1, rv0, rv1, wqt_s, wk_s, wvt_s,
            qt_s, k_ref, vt_ref, ctx_ref, wqkvt_ref, wobt_ref, pq_ref, kvt_ref, lhs_ref, e_ref, sems,
            *, S, M, D, Dc, H, HB, TQ, scale, variant, CB):
    L = 128
    HP = H // 2

    if True:
        cq = [
            pltpu.make_async_copy(wq_hbm.at[:, 0:L], rq0.at[0:M * H, :], sems.at[0]),
            pltpu.make_async_copy(wq_hbm.at[:, L:2 * L], rq1.at[0:M * H, :], sems.at[1]),
        ]
        ckv = [
            pltpu.make_async_copy(wuk_hbm.at[:, 0:L], rk0, sems.at[2]),
            pltpu.make_async_copy(wuk_hbm.at[:, L:2 * L], rk1, sems.at[3]),
            pltpu.make_async_copy(wuv_hbm.at[:, 0:L], rv0, sems.at[4]),
            pltpu.make_async_copy(wuv_hbm.at[:, L:2 * L], rv1, sems.at[5]),
        ]
        cc = pltpu.make_async_copy(c_hbm, c_ref, sems.at[6])
        cw = pltpu.make_async_copy(wot_hbm, wot_ref, sems.at[7])
        nb = S // CB
        cqkv = pltpu.make_async_copy(wqkv_hbm, wqkv_ref, sems.at[8])
        cgw = pltpu.make_async_copy(gw_hbm, gw_ref, sems.at[9])
        cwob = pltpu.make_async_copy(wob_hbm, wob_ref, sems.at[10])
        def xcopy(r):
            cs = pl.ds(pl.multiple_of(r * CB, CB), CB)
            return pltpu.make_async_copy(xt_hbm.at[:, cs], xt_ref.at[:, cs], xsems.at[r])
        cqkv.start()
        cgw.start()
        for r in range(nb if 'x0first' not in variant else 1):
            xcopy(r).start()
        if 'x0first' not in variant:
            cwob.start()
        if 'biglate' not in variant:
            for cp in cq + ckv + ([] if 'clate' in variant else [cc]):
                cp.start()

        rq0[M * H:, :] = jnp.zeros((rq0.shape[0] - M * H, L), _BF16)
        rq1[M * H:, :] = jnp.zeros((rq1.shape[0] - M * H, L), _BF16)

        Dh = M // HB
        kvt_ref[...] = jnp.zeros_like(kvt_ref)
        cqkv.wait()
        cgw.wait()
        if 'x0first' in variant:
            for r in range(1, nb):
                xcopy(r).start()
            cwob.start()
        if 'biglate' in variant and 'bigr' not in variant:
            for cp in cq + ckv + ([] if 'clate' in variant else [cc]):
                cp.start()
        if 'tnb1' in variant:
            gcol = jnp.broadcast_to(gw_ref[...].astype(_F32), (128, M)).T
        else:
            wqkvt_ref[0:3 * M, :] = wqkv_ref[...].T
            wqkvt_ref[3 * M:3 * M + 16, :] = jnp.broadcast_to(gw_ref[...], (16, M))

        def b1(r, carry):
            cs = pl.ds(pl.multiple_of(r * CB, CB), CB)
            xcopy(r).wait()
            if 'bigr' in variant:
                @pl.when(r == (1 if 'r1' in variant else 0))
                def _():
                    for cp in cq + ckv + ([] if 'clate' in variant else [cc]):
                        cp.start()
            if 'tnb1' in variant:
                xc = xt_ref[:, cs]
                qkvt = _tn(wqkv_ref[...], xc)
                gl = jnp.sum(xc.astype(_F32) * jnp.concatenate([gcol] * (CB // 128), axis=1), axis=0, keepdims=True)
                g_ref[:, cs] = jax.nn.sigmoid(gl)
            else:
                qkvt = _nn(wqkvt_ref[...], xt_ref[:, cs])
                g_ref[:, cs] = jax.nn.sigmoid(qkvt[3 * M:3 * M + 1, :])
            qk = qkvt[0:2 * M, :]
            pqk = (jnp.where(qk > 0, qk + 1.0, jnp.exp(qk)) + 1e-6).astype(_BF16)
            pq_ref[:, cs] = pqk[0:M, :]
            v_ext = jnp.concatenate([qkvt[2 * M:3 * M, :].astype(_BF16), jnp.ones((16, CB), _BF16)], axis=0)
            kvt_ref[...] += _nt(v_ext, pqk[M:2 * M, :])
            return carry
        jax.lax.fori_loop(0, S // CB, b1, 0)

        cwob.wait()
        wobt_ref[...] = wob_ref[...].T
        hr = jax.lax.broadcasted_iota(jnp.int32, (M, M), 0) // Dh
        hc = jax.lax.broadcasted_iota(jnp.int32, (M, M), 1) // Dh
        lhs_ref[0:M, :] = jnp.where(hr == hc, kvt_ref[0:M, :], 0.0).astype(_BF16)
        zr = jax.lax.broadcasted_iota(jnp.int32, (HB, M), 0)
        zc = jax.lax.broadcasted_iota(jnp.int32, (HB, M), 1) // Dh
        lhs_ref[M:M + HB, :] = jnp.where(zr == zc, kvt_ref[M:M + HB, :], 0.0).astype(_BF16)
        er = jax.lax.broadcasted_iota(jnp.int32, (M, 3 * HB), 0) // Dh
        ec = jax.lax.broadcasted_iota(jnp.int32, (M, 3 * HB), 1) % HB
        e_ref[...] = jnp.where(er == ec, 1.0, 0.0).astype(_BF16)

        def split(raw, r, i):
            view = raw.bitcast(jnp.uint32).at[pl.ds(pl.multiple_of(r * (L * HP), L * HP), L * HP), :]
            u = view[pl.ds(i, L, stride=HP), :]
            lo = pltpu.bitcast(u << 16, _F32)
            hi = pltpu.bitcast(u & jnp.uint32(0xFFFF0000), _F32)
            return lo, hi

        def ext_q(r):
            for i in range(HP):
                for j, rq in enumerate((rq0, rq1)):
                    lo, hi = split(rq, r, i)
                    wqt_s[2 * i, r, j * L:(j + 1) * L, :] = (lo * scale).T.astype(_BF16)
                    wqt_s[2 * i + 1, r, j * L:(j + 1) * L, :] = (hi * scale).T.astype(_BF16)

        def ext_kv(r):
            rs = pl.ds(pl.multiple_of(r * L, L), L)
            for i in range(HP):
                for j, (rk, rv) in enumerate(((rk0, rv0), (rk1, rv1))):
                    lo, hi = split(rk, r, i)
                    wk_s[2 * i, j, rs, :] = lo.astype(_BF16)
                    wk_s[2 * i + 1, j, rs, :] = hi.astype(_BF16)
                    lo, hi = split(rv, r, i)
                    wvt_s[2 * i, r, j * L:(j + 1) * L, :] = lo.T.astype(_BF16)
                    wvt_s[2 * i + 1, r, j * L:(j + 1) * L, :] = hi.T.astype(_BF16)

        for cp in cq:
            cp.wait()

        nqc = wqt_s.shape[1]
        assert nqc % nb == 0 or nb % nqc == 0
        def b2(r, carry):
            cs = pl.ds(pl.multiple_of(r * CB, CB), CB)
            nd = _nn(lhs_ref[...], pq_ref[:, cs])
            rc = 1.0 / (nd[M:M + HB, :] + 1e-6)
            r1 = rc.astype(_BF16)
            e1 = rc - r1.astype(_F32)
            r2 = e1.astype(_BF16)
            r3 = (e1 - r2.astype(_F32)).astype(_BF16)
            rx = _nn(e_ref[...], jnp.concatenate([r1, r2, r3], axis=0))
            ob = (nd[0:M, :] * rx).astype(_BF16)
            bt = _nn(wobt_ref[...], ob)
            acc_ref[:, cs] = (1.0 - g_ref[:, cs]) * bt
            for e in range(nqc // nb):
                ext_q(r * (nqc // nb) + e)
            return carry
        jax.lax.fori_loop(0, nb, b2, 0)

        for cp in ckv:
            cp.wait()
        if 'clate' in variant:
            cc.start()
        cw.start()

        nkc = Dc // L
        hpi = H // nkc
        def qall(r, carry):
            if 'qe0' in variant:
                ext_kv(r)
            for t in range(hpi):
                hh = r * hpi + t
                wq_h = jnp.concatenate([wqt_s[hh, t2] for t2 in range(nqc)], axis=1)[:, 0:M]
                qt_s[hh] = _nn(wq_h, xt_ref[...]).astype(_BF16)
                if 'qe1' in variant and t == 0:
                    ext_kv(r)
            if 'qe0' not in variant and 'qe1' not in variant:
                ext_kv(r)
            return carry
        jax.lax.fori_loop(0, nkc, qall, 0)
        cc.wait()
        cw.wait()

    def head(h, carry):
        k_ref[...] = _nn(c_ref[...], jnp.concatenate([wk_s[h, 0], wk_s[h, 1]], axis=1)).astype(_BF16)

        row = jax.lax.broadcasted_iota(jnp.int32, (TQ, TQ), 0)
        col = jax.lax.broadcasted_iota(jnp.int32, (TQ, TQ), 1)
        cmask = row <= col
        nq = S // TQ
        def scores(i):
            kv = (i + 1) * TQ
            s = _nn(k_ref[0:kv, :], qt_s[h, :, i * TQ:(i + 1) * TQ])
            sd = jnp.where(cmask, s[i * TQ:, :], -1e9)
            return (s[:i * TQ, :] if i > 0 else None), sd
        def smax(so, sd):
            m = jnp.max(sd, axis=0, keepdims=True)
            if so is not None:
                m = jnp.maximum(m, jnp.max(so, axis=0, keepdims=True))
            return m
        def sexp(so, sd, m):
            pd = jnp.exp(sd - m)
            l = jnp.sum(pd, axis=0, keepdims=True)
            if so is not None:
                po = jnp.exp(so - m)
                l = l + jnp.sum(po, axis=0, keepdims=True)
                p = jnp.concatenate([po.astype(_BF16), pd.astype(_BF16)], axis=0)
            else:
                p = pd.astype(_BF16)
            return p, l
        def pv(i, p, l):
            kv = (i + 1) * TQ
            r = g_ref[:, i * TQ:(i + 1) * TQ] / l
            ctx = _nn(vt_ref[:, 0:kv], p) * r
            ctx_ref[:, i * TQ:(i + 1) * TQ] = ctx.astype(_BF16)

        ss = [scores(j) for j in range(nq)]
        vt_ref[...] = _nt(jnp.concatenate([wvt_s[h, t2] for t2 in range(Dc // 128)], axis=1), c_ref[...]).astype(_BF16)
        m = smax(*ss[0])
        for i in range(nq):
            p, l = sexp(*ss[i], m)
            if i + 1 < nq:
                m = smax(*ss[i + 1])
            pv(i, p, l)

        acc_ref[...] += _nn(wot_ref[h], ctx_ref[...])

        return carry
    jax.lax.fori_loop(0, H, head, 0)
    o_ref[...] = acc_ref[...].astype(o_ref.dtype)

def build(TQ, variant, CB=512):
    @jax.jit
    def f(A_x, A_c_kv, A_w_q, A_w_uk, A_w_uv, A_w_o, B_x, B_wqkv, B_wo, gate_w):
        B, S, M = A_x.shape
        Sk, Dc = A_c_kv.shape[1], A_c_kv.shape[2]
        H, D = A_w_q.shape[1], A_w_q.shape[2]
        HB = 16
        MP = ((M + 127) // 128) * 128
        xt = A_x.reshape(S, M).T; c = A_c_kv.reshape(Sk, Dc)
        wq = A_w_q.reshape(M * H, D); wuk = A_w_uk.reshape(Dc * H, D); wuv = A_w_uv.reshape(Dc * H, D)
        wot = jnp.swapaxes(A_w_o, 1, 2); gw = gate_w.reshape(1, M)
        kern = functools.partial(_kernel, S=S, M=M, D=D, Dc=Dc, H=H, HB=HB, TQ=TQ, scale=float(D) ** -0.5, variant=variant, CB=CB)
        anyspec = pl.BlockSpec(memory_space=pl.ANY)
        out = pl.pallas_call(
            kern, grid=(1,),
            in_specs=[
                anyspec, anyspec, anyspec, anyspec,
                anyspec, anyspec, anyspec, anyspec, anyspec,
            ],
            out_specs=pl.BlockSpec((M, S), lambda h: (0, 0)),
            out_shape=jax.ShapeDtypeStruct((M, S), xt.dtype),
            scratch_shapes=[
                pltpu.VMEM((M, S), _BF16), pltpu.VMEM((M, 3 * M), _BF16), pltpu.VMEM((M, M), _BF16), pltpu.VMEM((1, M), _BF16),
                pltpu.SemaphoreType.DMA((S // CB,)),
                pltpu.VMEM((M, S), _F32), pltpu.VMEM((1, S), _F32),
                pltpu.VMEM((Sk, Dc), _BF16), pltpu.VMEM((H, M, D), _BF16),
                pltpu.VMEM((MP * H, 128), _BF16), pltpu.VMEM((MP * H, 128), _BF16),
                pltpu.VMEM((Dc * H, 128), _BF16), pltpu.VMEM((Dc * H, 128), _BF16),
                pltpu.VMEM((Dc * H, 128), _BF16), pltpu.VMEM((Dc * H, 128), _BF16),
                pltpu.VMEM((H, MP // 128, D, 128), _BF16), pltpu.VMEM((H, D // 128, Dc, 128), _BF16), pltpu.VMEM((H, Dc // 128, D, 128), _BF16),
                pltpu.VMEM((H, D, S), _BF16), pltpu.VMEM((Sk, D), _BF16), pltpu.VMEM((D, Sk), _BF16), pltpu.VMEM((D, S), _BF16),
                pltpu.VMEM((3 * M + 16, M), _BF16), pltpu.VMEM((M, M), _BF16), pltpu.VMEM((M, S), _BF16),
                pltpu.VMEM((M + 16, M), _F32), pltpu.VMEM((M + HB, M), _BF16), pltpu.VMEM((M, 3 * HB), _BF16),
                pltpu.SemaphoreType.DMA((11,)),
            ],
            compiler_params=pltpu.CompilerParams(dimension_semantics=("arbitrary",), vmem_limit_bytes=115 * 1024 * 1024),
        )(xt, B_wqkv, B_wo, gw, wot, c, wq, wuk, wuv)
        return out.T.reshape(B, S, M)
    return f


_impl = build(128, ('clate', 'biglate', 'bigr'))


@jax.jit
def pallas_gated_mix__compressed_kv_cla__linear_attn_block__prompt_kernel(
    A_x: jax.Array,
    A_c_kv: jax.Array,
    A_w_q: jax.Array,
    A_w_uk: jax.Array,
    A_w_uv: jax.Array,
    A_w_o: jax.Array,
    B_x: jax.Array,
    B_wqkv: jax.Array,
    B_wo: jax.Array,
    gate_w: jax.Array,
):
    return _impl(A_x, A_c_kv, A_w_q, A_w_uk, A_w_uv, A_w_o, B_x, B_wqkv, B_wo, gate_w)
```

```python
import functools

import jax
import jax.numpy as jnp
import jax.experimental.pallas as pl
import jax.experimental.pallas.tpu as pltpu

_F32 = jnp.float32
_BF16 = jnp.bfloat16
_L = 128


def _nt(a, b):
    return jax.lax.dot_general(a, b, (((1,), (1,)), ((), ())), preferred_element_type=_F32)


def _nn(a, b):
    return jnp.dot(a, b, preferred_element_type=_F32)


def _bd_ranges(M, Dh):
    out = []
    for d0 in range(0, M, _L):
        d1 = min(d0 + _L, M)
        e0 = (d0 // Dh) * Dh
        e1 = ((d1 - 1) // Dh + 1) * Dh
        out.append((d0, d1, (e0 // 16) * 16, min(-(-e1 // 16) * 16, M)))
    return out


def _kernel(xt_hbm, wqkv_hbm, wob_hbm, gw_hbm, wot_hbm, c_hbm, wq_hbm, wuk_hbm, wuv_hbm,
            o_ref,
            xt_ref, wqkv_ref, wob_ref, gw_ref, c_ref, wot_ref,
            rq0, rq1, rk0, rk1, rv0, rv1, wqt_s, wk_s, wvt_s, qt_s,
            acc_ref, g_ref, k_ref, vt_ref, ctx_ref,
            wqkvt_ref, pq_ref, kvt_ref, msk_ref, kvm_ref, gt_ref, z_ref, e_ref,
            sems, xsems, kvsems,
            *, S, M, D, Dc, H, HB, TQ, CB, scale, variant):
    L = _L
    HP = H // 2
    Dh = M // HB
    nb = S // CB
    nkc = Dc // L
    nqc = wqt_s.shape[1]
    RC = L * H

    cqkv = pltpu.make_async_copy(wqkv_hbm, wqkv_ref, sems.at[0])
    cgw = pltpu.make_async_copy(gw_hbm, gw_ref, sems.at[1])
    cwob = pltpu.make_async_copy(wob_hbm, wob_ref, sems.at[2])
    cq = [
        pltpu.make_async_copy(wq_hbm.at[:, 0:L], rq0.at[0:M * H, :], sems.at[3]),
        pltpu.make_async_copy(wq_hbm.at[:, L:2 * L], rq1.at[0:M * H, :], sems.at[4]),
    ]
    cc = pltpu.make_async_copy(c_hbm, c_ref, sems.at[5])
    cw = pltpu.make_async_copy(wot_hbm, wot_ref, sems.at[6])

    def xcopy(r):
        cs = pl.ds(pl.multiple_of(r * CB, CB), CB)
        return pltpu.make_async_copy(xt_hbm.at[:, cs], xt_ref.at[:, cs], xsems.at[r])

    def kvcopies(r):
        rs = pl.ds(pl.multiple_of(r * RC, RC), RC)
        return [
            pltpu.make_async_copy(wuk_hbm.at[rs, 0:L], rk0.at[rs, :], kvsems.at[4 * r]),
            pltpu.make_async_copy(wuk_hbm.at[rs, L:2 * L], rk1.at[rs, :], kvsems.at[4 * r + 1]),
            pltpu.make_async_copy(wuv_hbm.at[rs, 0:L], rv0.at[rs, :], kvsems.at[4 * r + 2]),
            pltpu.make_async_copy(wuv_hbm.at[rs, L:2 * L], rv1.at[rs, :], kvsems.at[4 * r + 3]),
        ]

    cqkv.start()
    cgw.start()
    for r in range(nb):
        xcopy(r).start()
    cwob.start()

    rq0[M * H:, :] = jnp.zeros((rq0.shape[0] - M * H, L), _BF16)
    rq1[M * H:, :] = jnp.zeros((rq1.shape[0] - M * H, L), _BF16)
    kvt_ref[...] = jnp.zeros_like(kvt_ref)
    kvm_ref[...] = jnp.zeros_like(kvm_ref)
    ranges = _bd_ranges(M, Dh)
    for t, (d0, d1, e0, e1) in enumerate(ranges):
        he = (jax.lax.broadcasted_iota(jnp.int32, (e1 - e0, d1 - d0), 0) + e0) // Dh
        hd = (jax.lax.broadcasted_iota(jnp.int32, (e1 - e0, d1 - d0), 1) + d0) // Dh
        msk_ref[t, 0:e1 - e0, 0:d1 - d0] = jnp.where(he == hd, 1, 0)
        zr = jax.lax.broadcasted_iota(jnp.int32, (HB, d1 - d0), 0)
        zd = (jax.lax.broadcasted_iota(jnp.int32, (HB, d1 - d0), 1) + d0) // Dh
        msk_ref[t, e1 - e0:e1 - e0 + HB, 0:d1 - d0] = jnp.where(zr == zd, 1, 0)
    er = jax.lax.broadcasted_iota(jnp.int32, (M, 3 * HB), 0) // Dh
    ec = jax.lax.broadcasted_iota(jnp.int32, (M, 3 * HB), 1) % HB
    e_ref[...] = jnp.where(er == ec, 1.0, 0.0).astype(_BF16)

    cqkv.wait()
    cgw.wait()
    for cp in cq:
        cp.start()
    wqkvt_ref[0:3 * M, :] = wqkv_ref[...].T
    wqkvt_ref[3 * M:3 * M + 16, :] = jnp.broadcast_to(gw_ref[...], (16, M))

    def b1(r, carry):
        cs = pl.ds(pl.multiple_of(r * CB, CB), CB)
        xcopy(r).wait()
        for e in range(nkc // nb):
            for cp in kvcopies(r * (nkc // nb) + e):
                cp.start()
        qkvt = _nn(wqkvt_ref[...], xt_ref[:, cs])
        g_ref[:, cs] = jax.nn.sigmoid(qkvt[3 * M:3 * M + 1, :])
        qk = qkvt[0:2 * M, :]
        pqk = (jnp.where(qk > 0, qk + 1.0, jnp.exp(qk)) + 1e-6).astype(_BF16)
        pq_ref[:, cs] = pqk[0:M, :]
        vt = qkvt[2 * M:3 * M, :].astype(_BF16)
        ones = jnp.ones((16, CB), _BF16)
        for t, (d0, d1, e0, e1) in enumerate(ranges):
            v_ext = jnp.concatenate([vt[e0:e1, :], ones], axis=0)
            kvt_ref[t, 0:e1 - e0 + 16, 0:d1 - d0] += _nt(v_ext, pqk[M + d0:M + d1, :])
        return carry
    jax.lax.fori_loop(0, nb, b1, 0)

    for t, (d0, d1, e0, e1) in enumerate(ranges):
        n = e1 - e0
        kz = jnp.where(msk_ref[t, 0:n + HB, 0:d1 - d0] != 0, kvt_ref[t, 0:n + HB, 0:d1 - d0], 0.0).astype(_BF16)
        kvm_ref[e0:e1, d0:d1] = kz[0:n, :]
        z_ref[:, d0:d1] = kz[n:n + HB, :]
    cwob.wait()
    gt_ref[...] = _nn(wob_ref[...].T, kvm_ref[...]).astype(_BF16)

    def split(raw, r, i):
        view = raw.bitcast(jnp.uint32).at[pl.ds(pl.multiple_of(r * (L * HP), L * HP), L * HP), :]
        u = view[pl.ds(i, L, stride=HP), :]
        lo = pltpu.bitcast(u << 16, _F32)
        hi = pltpu.bitcast(u & jnp.uint32(0xFFFF0000), _F32)
        return lo, hi

    def ext_q(r):
        for i in range(HP):
            for j, rq in enumerate((rq0, rq1)):
                lo, hi = split(rq, r, i)
                wqt_s[2 * i, r, j * L:(j + 1) * L, :] = (lo * scale).T.astype(_BF16)
                wqt_s[2 * i + 1, r, j * L:(j + 1) * L, :] = (hi * scale).T.astype(_BF16)

    def ext_kv(r):
        rs = pl.ds(pl.multiple_of(r * L, L), L)
        for i in range(HP):
            for j, (rk, rv) in enumerate(((rk0, rv0), (rk1, rv1))):
                lo, hi = split(rk, r, i)
                wk_s[2 * i, j, rs, :] = lo.astype(_BF16)
                wk_s[2 * i + 1, j, rs, :] = hi.astype(_BF16)
                lo, hi = split(rv, r, i)
                wvt_s[2 * i, r, j * L:(j + 1) * L, :] = lo.T.astype(_BF16)
                wvt_s[2 * i + 1, r, j * L:(j + 1) * L, :] = hi.T.astype(_BF16)

    for cp in cq:
        cp.wait()

    def b2(r, carry):
        cs = pl.ds(pl.multiple_of(r * CB, CB), CB)
        pq = pq_ref[:, cs]
        rc = 1.0 / (_nn(z_ref[...], pq) + 1e-6)
        r1 = rc.astype(_BF16)
        e1 = rc - r1.astype(_F32)
        r2 = e1.astype(_BF16)
        r3 = (e1 - r2.astype(_F32)).astype(_BF16)
        rx = _nn(e_ref[...], jnp.concatenate([r1, r2, r3], axis=0))
        pr = (pq.astype(_F32) * rx).astype(_BF16)
        acc_ref[:, cs] = (1.0 - g_ref[:, cs]) * _nn(gt_ref[...], pr)
        for e in range(nqc // nb):
            ext_q(r * (nqc // nb) + e)
        return carry
    jax.lax.fori_loop(0, nb, b2, 0)

    cc.start()
    cw.start()

    hpi = H // nkc

    def qall(r, carry):
        for cp in kvcopies(r):
            cp.wait()
        for t in range(hpi):
            hh = r * hpi + t
            wq_h = jnp.concatenate([wqt_s[hh, t2] for t2 in range(nqc)], axis=1)[:, 0:M]
            qt_s[hh] = _nn(wq_h, xt_ref[...]).astype(_BF16)
        ext_kv(r)
        return carry
    jax.lax.fori_loop(0, nkc, qall, 0)
    cc.wait()
    cw.wait()

    row = jax.lax.broadcasted_iota(jnp.int32, (TQ, TQ), 0)
    col = jax.lax.broadcasted_iota(jnp.int32, (TQ, TQ), 1)
    cmask = row <= col
    nq = S // TQ

    def head(h, carry):
        k_ref[...] = _nn(c_ref[...], jnp.concatenate([wk_s[h, j] for j in range(D // L)], axis=1)).astype(_BF16)

        def scores(i):
            kv = (i + 1) * TQ
            s = _nn(k_ref[0:kv, :], qt_s[h, :, i * TQ:(i + 1) * TQ])
            sd = jnp.where(cmask, s[i * TQ:, :], -1e9)
            return (s[:i * TQ, :] if i > 0 else None), sd

        def smax(so, sd):
            m = jnp.max(sd, axis=0, keepdims=True)
            if so is not None:
                m = jnp.maximum(m, jnp.max(so, axis=0, keepdims=True))
            return m

        def sexp(so, sd, m):
            pd = jnp.exp(sd - m)
            l = jnp.sum(pd, axis=0, keepdims=True)
            if so is not None:
                po = jnp.exp(so - m)
                l = l + jnp.sum(po, axis=0, keepdims=True)
                p = jnp.concatenate([po.astype(_BF16), pd.astype(_BF16)], axis=0)
            else:
                p = pd.astype(_BF16)
            return p, l

        def pv(i, p, l):
            kv = (i + 1) * TQ
            r = g_ref[:, i * TQ:(i + 1) * TQ] / l
            ctx = _nn(vt_ref[:, 0:kv], p) * r
            ctx_ref[:, i * TQ:(i + 1) * TQ] = ctx.astype(_BF16)

        ss = [scores(j) for j in range(nq)]
        vt_ref[...] = _nt(jnp.concatenate([wvt_s[h, t2] for t2 in range(nkc)], axis=1), c_ref[...]).astype(_BF16)
        m = smax(*ss[0])
        for i in range(nq):
            p, l = sexp(*ss[i], m)
            if i + 1 < nq:
                m = smax(*ss[i + 1])
            pv(i, p, l)

        acc_ref[...] += _nn(wot_ref[h], ctx_ref[...])
        return carry
    jax.lax.fori_loop(0, H, head, 0)

    o_ref[...] = acc_ref[...].astype(o_ref.dtype)


def build(TQ, variant, CB=512):
    @jax.jit
    def f(A_x, A_c_kv, A_w_q, A_w_uk, A_w_uv, A_w_o, B_x, B_wqkv, B_wo, gate_w):
        B, S, M = A_x.shape
        Sk, Dc = A_c_kv.shape[1], A_c_kv.shape[2]
        H, D = A_w_q.shape[1], A_w_q.shape[2]
        assert B == 1 and S == Sk and D == 2 * _L
        HB = 16
        L = _L
        MP = -(-M // L) * L
        xt = A_x.reshape(S, M).T
        c = A_c_kv.reshape(Sk, Dc)
        wq = A_w_q.reshape(M * H, D)
        wuk = A_w_uk.reshape(Dc * H, D)
        wuv = A_w_uv.reshape(Dc * H, D)
        wot = jnp.swapaxes(A_w_o, 1, 2)
        gw = gate_w.reshape(1, M)
        ranges = _bd_ranges(M, M // HB)
        kvrows = max(e1 - e0 for _, _, e0, e1 in ranges) + 16
        kern = functools.partial(_kernel, S=S, M=M, D=D, Dc=Dc, H=H, HB=HB, TQ=TQ, CB=CB,
                                 scale=float(D) ** -0.5, variant=variant)
        anyspec = pl.BlockSpec(memory_space=pl.ANY)
        out = pl.pallas_call(
            kern, grid=(1,),
            in_specs=[anyspec] * 9,
            out_specs=pl.BlockSpec((M, S), lambda i: (0, 0)),
            out_shape=jax.ShapeDtypeStruct((M, S), xt.dtype),
            scratch_shapes=[
                pltpu.VMEM((M, S), _BF16), pltpu.VMEM((M, 3 * M), _BF16), pltpu.VMEM((M, M), _BF16),
                pltpu.VMEM((1, M), _BF16), pltpu.VMEM((Sk, Dc), _BF16), pltpu.VMEM((H, M, D), _BF16),
                pltpu.VMEM((MP * H, L), _BF16), pltpu.VMEM((MP * H, L), _BF16),
                pltpu.VMEM((Dc * H, L), _BF16), pltpu.VMEM((Dc * H, L), _BF16),
                pltpu.VMEM((Dc * H, L), _BF16), pltpu.VMEM((Dc * H, L), _BF16),
                pltpu.VMEM((H, MP // L, D, L), _BF16), pltpu.VMEM((H, D // L, Dc, L), _BF16),
                pltpu.VMEM((H, Dc // L, D, L), _BF16), pltpu.VMEM((H, D, S), _BF16),
                pltpu.VMEM((M, S), _F32), pltpu.VMEM((1, S), _F32),
                pltpu.VMEM((Sk, D), _BF16), pltpu.VMEM((D, Sk), _BF16), pltpu.VMEM((D, S), _BF16),
                pltpu.VMEM((3 * M + 16, M), _BF16), pltpu.VMEM((M, S), _BF16),
                pltpu.VMEM((len(ranges), kvrows, L), _F32), pltpu.VMEM((len(ranges), kvrows, L), jnp.int32), pltpu.VMEM((M, M), _BF16), pltpu.VMEM((M, M), _BF16),
                pltpu.VMEM((HB, M), _BF16), pltpu.VMEM((M, 3 * HB), _BF16),
                pltpu.SemaphoreType.DMA((7,)), pltpu.SemaphoreType.DMA((S // CB,)),
                pltpu.SemaphoreType.DMA((4 * (Dc // L),)),
            ],
            compiler_params=pltpu.CompilerParams(dimension_semantics=("arbitrary",),
                                                 vmem_limit_bytes=115 * 1024 * 1024),
        )(xt, B_wqkv, B_wo, gw, wot, c, wq, wuk, wuv)
        return out.T.reshape(B, S, M)
    return f


_impl = build(128, ())


@jax.jit
def pallas_gated_mix__compressed_kv_cla__linear_attn_block__prompt_kernel(
    A_x: jax.Array,
    A_c_kv: jax.Array,
    A_w_q: jax.Array,
    A_w_uk: jax.Array,
    A_w_uv: jax.Array,
    A_w_o: jax.Array,
    B_x: jax.Array,
    B_wqkv: jax.Array,
    B_wo: jax.Array,
    gate_w: jax.Array,
):
    return _impl(A_x, A_c_kv, A_w_q, A_w_uk, A_w_uv, A_w_o, B_x, B_wqkv, B_wo, gate_w)
```

```python
import functools

import jax
import jax.numpy as jnp
import jax.experimental.pallas as pl
import jax.experimental.pallas.tpu as pltpu

_F32 = jnp.float32
_BF16 = jnp.bfloat16
_L = 128


def _nt(a, b):
    return jax.lax.dot_general(a, b, (((1,), (1,)), ((), ())), preferred_element_type=_F32)


def _nn(a, b):
    return jnp.dot(a, b, preferred_element_type=_F32)


def _bd_ranges(M, Dh):
    out = []
    for d0 in range(0, M, _L):
        d1 = min(d0 + _L, M)
        e0 = (d0 // Dh) * Dh
        e1 = ((d1 - 1) // Dh + 1) * Dh
        out.append((d0, d1, (e0 // 16) * 16, min(-(-e1 // 16) * 16, M)))
    return out


def _kernel(xt_hbm, wqkv_hbm, wob_hbm, gw_hbm, wot_hbm, c_hbm, wq_hbm, wuk_hbm, wuv_hbm,
            o_ref,
            xt_ref, wqkv_ref, wob_ref, gw_ref, c_ref, wot_ref,
            rq0, rq1, rka0, rka1, rva0, rva1, rkb0, rkb1, rvb0, rvb1, wqt_s, wk_s, wvt_s, qt_s,
            acc_ref, g_ref, k_ref, vt_ref, ctx_ref,
            wqkvt_ref, pq_ref, kvt_ref, msk_ref, kvm_ref, gt_ref, z_ref, e_ref,
            sems, xsems, kvsems,
            *, S, M, D, Dc, H, HB, TQ, CB, scale):
    L = _L
    HP = H // 2
    Dh = M // HB
    nb = S // CB
    nkc = Dc // L
    nqc = wqt_s.shape[1]

    cqkv = pltpu.make_async_copy(wqkv_hbm, wqkv_ref, sems.at[0])
    cgw = pltpu.make_async_copy(gw_hbm, gw_ref, sems.at[1])
    cwob = pltpu.make_async_copy(wob_hbm, wob_ref, sems.at[2])
    cq = [
        pltpu.make_async_copy(wq_hbm.at[:, 0:L], rq0.at[0:M * H, :], sems.at[3]),
        pltpu.make_async_copy(wq_hbm.at[:, L:2 * L], rq1.at[0:M * H, :], sems.at[4]),
    ]
    cc = pltpu.make_async_copy(c_hbm, c_ref, sems.at[5])
    cw = pltpu.make_async_copy(wot_hbm, wot_ref, sems.at[6])

    def xcopy(r):
        cs = pl.ds(pl.multiple_of(r * CB, CB), CB)
        return pltpu.make_async_copy(xt_hbm.at[:, cs], xt_ref.at[:, cs], xsems.at[r])

    GR = (Dc // 2) * H
    kvraw = ((rka0, rka1, rva0, rva1), (rkb0, rkb1, rvb0, rvb1))

    def kvcopies(gi):
        rs = pl.ds(gi * GR, GR)
        k0, k1, v0, v1 = kvraw[gi]
        return [
            pltpu.make_async_copy(wuk_hbm.at[rs, 0:L], k0, kvsems.at[4 * gi]),
            pltpu.make_async_copy(wuk_hbm.at[rs, L:2 * L], k1, kvsems.at[4 * gi + 1]),
            pltpu.make_async_copy(wuv_hbm.at[rs, 0:L], v0, kvsems.at[4 * gi + 2]),
            pltpu.make_async_copy(wuv_hbm.at[rs, L:2 * L], v1, kvsems.at[4 * gi + 3]),
        ]

    cqkv.start()
    cgw.start()
    for r in range(nb):
        xcopy(r).start()
    cwob.start()

    rq0[M * H:, :] = jnp.zeros((rq0.shape[0] - M * H, L), _BF16)
    rq1[M * H:, :] = jnp.zeros((rq1.shape[0] - M * H, L), _BF16)
    kvt_ref[...] = jnp.zeros_like(kvt_ref)
    kvm_ref[...] = jnp.zeros_like(kvm_ref)
    ranges = _bd_ranges(M, Dh)
    for t, (d0, d1, e0, e1) in enumerate(ranges):
        he = (jax.lax.broadcasted_iota(jnp.int32, (e1 - e0, d1 - d0), 0) + e0) // Dh
        hd = (jax.lax.broadcasted_iota(jnp.int32, (e1 - e0, d1 - d0), 1) + d0) // Dh
        msk_ref[t, 0:e1 - e0, 0:d1 - d0] = jnp.where(he == hd, 1, 0)
        zr = jax.lax.broadcasted_iota(jnp.int32, (HB, d1 - d0), 0)
        zd = (jax.lax.broadcasted_iota(jnp.int32, (HB, d1 - d0), 1) + d0) // Dh
        msk_ref[t, e1 - e0:e1 - e0 + HB, 0:d1 - d0] = jnp.where(zr == zd, 1, 0)
    er = jax.lax.broadcasted_iota(jnp.int32, (M, 3 * HB), 0) // Dh
    ec = jax.lax.broadcasted_iota(jnp.int32, (M, 3 * HB), 1) % HB
    e_ref[...] = jnp.where(er == ec, 1.0, 0.0).astype(_BF16)

    cqkv.wait()
    cgw.wait()
    for cp in cq:
        cp.start()
    wqkvt_ref[0:3 * M, :] = wqkv_ref[...].T
    wqkvt_ref[3 * M:3 * M + 16, :] = jnp.broadcast_to(gw_ref[...], (16, M))

    def b1(r, carry):
        cs = pl.ds(pl.multiple_of(r * CB, CB), CB)
        xcopy(r).wait()
        for gi in range(2):
            @pl.when(r == gi * (nb // 2))
            def _():
                for cp in kvcopies(gi):
                    cp.start()
        qkvt = _nn(wqkvt_ref[...], xt_ref[:, cs])
        g_ref[:, cs] = jax.nn.sigmoid(qkvt[3 * M:3 * M + 1, :])
        qk = qkvt[0:2 * M, :]
        pqk = (jnp.where(qk > 0, qk + 1.0, jnp.exp(qk)) + 1e-6).astype(_BF16)
        pq_ref[:, cs] = pqk[0:M, :]
        vt = qkvt[2 * M:3 * M, :].astype(_BF16)
        ones = jnp.ones((16, CB), _BF16)
        for t, (d0, d1, e0, e1) in enumerate(ranges):
            v_ext = jnp.concatenate([vt[e0:e1, :], ones], axis=0)
            kvt_ref[t, 0:e1 - e0 + 16, 0:d1 - d0] += _nt(v_ext, pqk[M + d0:M + d1, :])
        return carry
    jax.lax.fori_loop(0, nb, b1, 0)

    for t, (d0, d1, e0, e1) in enumerate(ranges):
        n = e1 - e0
        kz = jnp.where(msk_ref[t, 0:n + HB, 0:d1 - d0] != 0, kvt_ref[t, 0:n + HB, 0:d1 - d0], 0.0).astype(_BF16)
        kvm_ref[e0:e1, d0:d1] = kz[0:n, :]
        z_ref[:, d0:d1] = kz[n:n + HB, :]
    cwob.wait()
    gt_ref[...] = _nn(wob_ref[...].T, kvm_ref[...]).astype(_BF16)

    def split(raw, r, i):
        view = raw.bitcast(jnp.uint32).at[pl.ds(pl.multiple_of(r * (L * HP), L * HP), L * HP), :]
        u = view[pl.ds(i, L, stride=HP), :]
        lo = pltpu.bitcast(u << 16, _F32)
        hi = pltpu.bitcast(u & jnp.uint32(0xFFFF0000), _F32)
        return lo, hi

    def ext_q(r):
        for i in range(HP):
            for j, rq in enumerate((rq0, rq1)):
                lo, hi = split(rq, r, i)
                wqt_s[2 * i, r, j * L:(j + 1) * L, :] = (lo * scale).T.astype(_BF16)
                wqt_s[2 * i + 1, r, j * L:(j + 1) * L, :] = (hi * scale).T.astype(_BF16)

    def ext_kv(gi, rr):
        r = gi * (nkc // 2) + rr
        rs = pl.ds(pl.multiple_of(r * L, L), L)
        k0, k1, v0, v1 = kvraw[gi]
        for i in range(HP):
            for j, (rk, rv) in enumerate(((k0, v0), (k1, v1))):
                lo, hi = split(rk, rr, i)
                wk_s[2 * i, j, rs, :] = lo.astype(_BF16)
                wk_s[2 * i + 1, j, rs, :] = hi.astype(_BF16)
                lo, hi = split(rv, rr, i)
                wvt_s[2 * i, r, j * L:(j + 1) * L, :] = lo.T.astype(_BF16)
                wvt_s[2 * i + 1, r, j * L:(j + 1) * L, :] = hi.T.astype(_BF16)

    for cp in cq:
        cp.wait()

    def b2(r, carry):
        cs = pl.ds(pl.multiple_of(r * CB, CB), CB)
        pq = pq_ref[:, cs]
        rc = 1.0 / (_nn(z_ref[...], pq) + 1e-6)
        r1 = rc.astype(_BF16)
        e1 = rc - r1.astype(_F32)
        r2 = e1.astype(_BF16)
        r3 = (e1 - r2.astype(_F32)).astype(_BF16)
        rx = _nn(e_ref[...], jnp.concatenate([r1, r2, r3], axis=0))
        pr = (pq.astype(_F32) * rx).astype(_BF16)
        acc_ref[:, cs] = (1.0 - g_ref[:, cs]) * _nn(gt_ref[...], pr)
        for e in range(nqc // nb):
            ext_q(r * (nqc // nb) + e)
        return carry
    jax.lax.fori_loop(0, nb, b2, 0)

    cc.start()
    cw.start()

    hpi = H // nkc

    for gi in range(2):
        for cp in kvcopies(gi):
            cp.wait()

        def qall(rr, carry, gi=gi):
            for t in range(hpi):
                hh = (gi * (nkc // 2) + rr) * hpi + t
                wq_h = jnp.concatenate([wqt_s[hh, t2] for t2 in range(nqc)], axis=1)[:, 0:M]
                qt_s[hh] = _nn(wq_h, xt_ref[...]).astype(_BF16)
            ext_kv(gi, rr)
            return carry
        jax.lax.fori_loop(0, nkc // 2, qall, 0)
    cc.wait()
    cw.wait()

    row = jax.lax.broadcasted_iota(jnp.int32, (TQ, TQ), 0)
    col = jax.lax.broadcasted_iota(jnp.int32, (TQ, TQ), 1)
    cmask = row <= col
    nq = S // TQ

    def head(h, carry):
        k_ref[...] = _nn(c_ref[...], jnp.concatenate([wk_s[h, j] for j in range(D // L)], axis=1)).astype(_BF16)

        def scores(i):
            kv = (i + 1) * TQ
            s = _nn(k_ref[0:kv, :], qt_s[h, :, i * TQ:(i + 1) * TQ])
            sd = jnp.where(cmask, s[i * TQ:, :], -1e9)
            return (s[:i * TQ, :] if i > 0 else None), sd

        def smax(so, sd):
            m = jnp.max(sd, axis=0, keepdims=True)
            if so is not None:
                m = jnp.maximum(m, jnp.max(so, axis=0, keepdims=True))
            return m

        def sexp(so, sd, m):
            pd = jnp.exp(sd - m)
            l = jnp.sum(pd, axis=0, keepdims=True)
            if so is not None:
                po = jnp.exp(so - m)
                l = l + jnp.sum(po, axis=0, keepdims=True)
                p = jnp.concatenate([po.astype(_BF16), pd.astype(_BF16)], axis=0)
            else:
                p = pd.astype(_BF16)
            return p, l

        def pv(i, p, l):
            kv = (i + 1) * TQ
            r = g_ref[:, i * TQ:(i + 1) * TQ] / l
            ctx = _nn(vt_ref[:, 0:kv], p) * r
            ctx_ref[:, i * TQ:(i + 1) * TQ] = ctx.astype(_BF16)

        ss = [scores(j) for j in range(nq)]
        vt_ref[...] = _nt(jnp.concatenate([wvt_s[h, t2] for t2 in range(nkc)], axis=1), c_ref[...]).astype(_BF16)
        m = smax(*ss[0])
        for i in range(nq):
            p, l = sexp(*ss[i], m)
            if i + 1 < nq:
                m = smax(*ss[i + 1])
            pv(i, p, l)

        acc_ref[...] += _nn(wot_ref[h], ctx_ref[...])
        return carry
    jax.lax.fori_loop(0, H, head, 0)

    o_ref[...] = acc_ref[...].astype(o_ref.dtype)


@jax.jit
def pallas_gated_mix__compressed_kv_cla__linear_attn_block__prompt_kernel(
    A_x: jax.Array,
    A_c_kv: jax.Array,
    A_w_q: jax.Array,
    A_w_uk: jax.Array,
    A_w_uv: jax.Array,
    A_w_o: jax.Array,
    B_x: jax.Array,
    B_wqkv: jax.Array,
    B_wo: jax.Array,
    gate_w: jax.Array,
):
    B, S, M = A_x.shape
    Sk, Dc = A_c_kv.shape[1], A_c_kv.shape[2]
    H, D = A_w_q.shape[1], A_w_q.shape[2]
    L = _L
    HB = 16
    TQ = L
    CB = 512
    assert B == 1 and S == Sk and D == 2 * L
    MP = -(-M // L) * L

    xt = A_x.reshape(S, M).T
    c = A_c_kv.reshape(Sk, Dc)
    wq = A_w_q.reshape(M * H, D)
    wuk = A_w_uk.reshape(Dc * H, D)
    wuv = A_w_uv.reshape(Dc * H, D)
    wot = jnp.swapaxes(A_w_o, 1, 2)
    gw = gate_w.reshape(1, M)

    ranges = _bd_ranges(M, M // HB)
    kvrows = max(e1 - e0 for _, _, e0, e1 in ranges) + 16
    kern = functools.partial(_kernel, S=S, M=M, D=D, Dc=Dc, H=H, HB=HB, TQ=TQ, CB=CB,
                             scale=float(D) ** -0.5)
    out = pl.pallas_call(
        kern,
        grid=(1,),
        in_specs=[pl.BlockSpec(memory_space=pl.ANY)] * 9,
        out_specs=pl.BlockSpec((M, S), lambda i: (0, 0)),
        out_shape=jax.ShapeDtypeStruct((M, S), xt.dtype),
        scratch_shapes=[
            pltpu.VMEM((M, S), _BF16), pltpu.VMEM((M, 3 * M), _BF16), pltpu.VMEM((M, M), _BF16),
            pltpu.VMEM((1, M), _BF16), pltpu.VMEM((Sk, Dc), _BF16), pltpu.VMEM((H, M, D), _BF16),
            pltpu.VMEM((MP * H, L), _BF16), pltpu.VMEM((MP * H, L), _BF16),
            *[pltpu.VMEM((Dc * H // 2, L), _BF16) for _ in range(8)],
            pltpu.VMEM((H, MP // L, D, L), _BF16), pltpu.VMEM((H, D // L, Dc, L), _BF16),
            pltpu.VMEM((H, Dc // L, D, L), _BF16), pltpu.VMEM((H, D, S), _BF16),
            pltpu.VMEM((M, S), _F32), pltpu.VMEM((1, S), _F32),
            pltpu.VMEM((Sk, D), _BF16), pltpu.VMEM((D, Sk), _BF16), pltpu.VMEM((D, S), _BF16),
            pltpu.VMEM((3 * M + 16, M), _BF16), pltpu.VMEM((M, S), _BF16),
            pltpu.VMEM((len(ranges), kvrows, L), _F32), pltpu.VMEM((len(ranges), kvrows, L), jnp.int32),
            pltpu.VMEM((M, M), _BF16), pltpu.VMEM((M, M), _BF16),
            pltpu.VMEM((HB, M), _BF16), pltpu.VMEM((M, 3 * HB), _BF16),
            pltpu.SemaphoreType.DMA((7,)), pltpu.SemaphoreType.DMA((S // CB,)),
            pltpu.SemaphoreType.DMA((8,)),
        ],
        compiler_params=pltpu.CompilerParams(
            dimension_semantics=("arbitrary",),
            vmem_limit_bytes=115 * 1024 * 1024,
        ),
    )(xt, B_wqkv, B_wo, gw, wot, c, wq, wuk, wuv)
    return out.T.reshape(B, S, M)
```

```python
import functools

import jax
import jax.numpy as jnp
import jax.experimental.pallas as pl
import jax.experimental.pallas.tpu as pltpu

_F32 = jnp.float32
_BF16 = jnp.bfloat16
_L = 128


def _nt(a, b):
    return jax.lax.dot_general(a, b, (((1,), (1,)), ((), ())), preferred_element_type=_F32)


def _nn(a, b):
    return jnp.dot(a, b, preferred_element_type=_F32)


def _bd_ranges(M, Dh):
    out = []
    for d0 in range(0, M, _L):
        d1 = min(d0 + _L, M)
        e0 = (d0 // Dh) * Dh
        e1 = ((d1 - 1) // Dh + 1) * Dh
        out.append((d0, d1, (e0 // 16) * 16, min(-(-e1 // 16) * 16, M)))
    return out


def _kernel(xt_hbm, wqkv_hbm, wob_hbm, gw_hbm, wot_hbm, c_hbm, wq_hbm, wuk_hbm, wuv_hbm,
            o_ref,
            xt_ref, wqkv_ref, wob_ref, gw_ref, c_ref, wot_ref,
            rq0, rq1, rka0, rka1, rva0, rva1, rkb0, rkb1, rvb0, rvb1, wall, qt_s,
            acc_ref, g_ref, k_ref, vt_ref, ctx_ref,
            wqkvt_ref, pq_ref, kvt_ref, msk_ref, kvm_ref, gt_ref, z_ref, e_ref,
            sems, xsems, kvsems,
            *, S, M, D, Dc, H, HB, TQ, CB, scale):
    L = _L
    HP = H // 2
    Dh = M // HB
    nb = S // CB
    nkc = Dc // L
    nqc = -(-M // L)
    KB = Dc // D
    QOFF, KOFF, VOFF = 0, H * nqc, H * nqc + H * (D // L) * KB

    cqkv = pltpu.make_async_copy(wqkv_hbm, wqkv_ref, sems.at[0])
    cgw = pltpu.make_async_copy(gw_hbm, gw_ref, sems.at[1])
    cwob = pltpu.make_async_copy(wob_hbm, wob_ref, sems.at[2])
    cq = [
        pltpu.make_async_copy(wq_hbm.at[:, 0:L], rq0.at[0:M * H, :], sems.at[3]),
        pltpu.make_async_copy(wq_hbm.at[:, L:2 * L], rq1.at[0:M * H, :], sems.at[4]),
    ]
    cc = pltpu.make_async_copy(c_hbm, c_ref, sems.at[5])
    cw = pltpu.make_async_copy(wot_hbm, wot_ref, sems.at[6])

    def xcopy(r):
        cs = pl.ds(pl.multiple_of(r * CB, CB), CB)
        return pltpu.make_async_copy(xt_hbm.at[:, cs], xt_ref.at[:, cs], xsems.at[r])

    GR = (Dc // 2) * H
    kvraw = ((rka0, rka1, rva0, rva1), (rkb0, rkb1, rvb0, rvb1))

    def kvcopies(gi):
        rs = pl.ds(gi * GR, GR)
        k0, k1, v0, v1 = kvraw[gi]
        return [
            pltpu.make_async_copy(wuk_hbm.at[rs, 0:L], k0, kvsems.at[4 * gi]),
            pltpu.make_async_copy(wuk_hbm.at[rs, L:2 * L], k1, kvsems.at[4 * gi + 1]),
            pltpu.make_async_copy(wuv_hbm.at[rs, 0:L], v0, kvsems.at[4 * gi + 2]),
            pltpu.make_async_copy(wuv_hbm.at[rs, L:2 * L], v1, kvsems.at[4 * gi + 3]),
        ]

    cqkv.start()
    cgw.start()
    for r in range(nb):
        xcopy(r).start()
    cwob.start()

    rq0[M * H:, :] = jnp.zeros((rq0.shape[0] - M * H, L), _BF16)
    rq1[M * H:, :] = jnp.zeros((rq1.shape[0] - M * H, L), _BF16)
    kvt_ref[...] = jnp.zeros_like(kvt_ref)
    kvm_ref[...] = jnp.zeros_like(kvm_ref)
    ranges = _bd_ranges(M, Dh)
    for t, (d0, d1, e0, e1) in enumerate(ranges):
        he = (jax.lax.broadcasted_iota(jnp.int32, (e1 - e0, d1 - d0), 0) + e0) // Dh
        hd = (jax.lax.broadcasted_iota(jnp.int32, (e1 - e0, d1 - d0), 1) + d0) // Dh
        msk_ref[t, 0:e1 - e0, 0:d1 - d0] = jnp.where(he == hd, 1, 0)
        zr = jax.lax.broadcasted_iota(jnp.int32, (HB, d1 - d0), 0)
        zd = (jax.lax.broadcasted_iota(jnp.int32, (HB, d1 - d0), 1) + d0) // Dh
        msk_ref[t, e1 - e0:e1 - e0 + HB, 0:d1 - d0] = jnp.where(zr == zd, 1, 0)
    er = jax.lax.broadcasted_iota(jnp.int32, (M, 3 * HB), 0) // Dh
    ec = jax.lax.broadcasted_iota(jnp.int32, (M, 3 * HB), 1) % HB
    e_ref[...] = jnp.where(er == ec, 1.0, 0.0).astype(_BF16)

    cqkv.wait()
    cgw.wait()
    for cp in cq:
        cp.start()
    wqkvt_ref[0:3 * M, :] = wqkv_ref[...].T
    wqkvt_ref[3 * M:3 * M + 16, :] = jnp.broadcast_to(gw_ref[...], (16, M))

    def b1(r, carry):
        cs = pl.ds(pl.multiple_of(r * CB, CB), CB)
        xcopy(r).wait()
        for gi in range(2):
            @pl.when(r == gi * (nb // 2))
            def _():
                for cp in kvcopies(gi):
                    cp.start()
        qkvt = _nn(wqkvt_ref[...], xt_ref[:, cs])
        g_ref[:, cs] = jax.nn.sigmoid(qkvt[3 * M:3 * M + 1, :])
        qk = qkvt[0:2 * M, :]
        pqk = (jnp.where(qk > 0, qk + 1.0, jnp.exp(qk)) + 1e-6).astype(_BF16)
        pq_ref[:, cs] = pqk[0:M, :]
        vt = qkvt[2 * M:3 * M, :].astype(_BF16)
        ones = jnp.ones((16, CB), _BF16)
        for t, (d0, d1, e0, e1) in enumerate(ranges):
            v_ext = jnp.concatenate([vt[e0:e1, :], ones], axis=0)
            kvt_ref[t, 0:e1 - e0 + 16, 0:d1 - d0] += _nt(v_ext, pqk[M + d0:M + d1, :])
        return carry
    jax.lax.fori_loop(0, nb, b1, 0)

    for t, (d0, d1, e0, e1) in enumerate(ranges):
        n = e1 - e0
        kz = jnp.where(msk_ref[t, 0:n + HB, 0:d1 - d0] != 0, kvt_ref[t, 0:n + HB, 0:d1 - d0], 0.0).astype(_BF16)
        kvm_ref[e0:e1, d0:d1] = kz[0:n, :]
        z_ref[:, d0:d1] = kz[n:n + HB, :]
    cwob.wait()
    gt_ref[...] = _nn(wob_ref[...].T, kvm_ref[...]).astype(_BF16)

    def split(raw, r, i):
        view = raw.bitcast(jnp.uint32).at[pl.ds(pl.multiple_of(r * (L * HP), L * HP), L * HP), :]
        u = view[pl.ds(i, L, stride=HP), :]
        lo = pltpu.bitcast(u << 16, _F32)
        hi = pltpu.bitcast(u & jnp.uint32(0xFFFF0000), _F32)
        return lo, hi

    def ext_q(r):
        for i in range(HP):
            for j, rq in enumerate((rq0, rq1)):
                lo, hi = split(rq, r, i)
                wall[QOFF + 2 * i * nqc + r, j * L:(j + 1) * L, :] = (lo * scale).T.astype(_BF16)
                wall[QOFF + (2 * i + 1) * nqc + r, j * L:(j + 1) * L, :] = (hi * scale).T.astype(_BF16)

    def ext_kv(gi, rr):
        r = gi * (nkc // 2) + rr
        kb = r // (D // L)
        ks = pl.ds(pl.multiple_of((r % (D // L)) * L, L), L)
        k0, k1, v0, v1 = kvraw[gi]
        for i in range(HP):
            for j, (rk, rv) in enumerate(((k0, v0), (k1, v1))):
                lo, hi = split(rk, rr, i)
                wall[KOFF + ((2 * i) * (D // L) + j) * KB + kb, ks, :] = lo.astype(_BF16)
                wall[KOFF + ((2 * i + 1) * (D // L) + j) * KB + kb, ks, :] = hi.astype(_BF16)
                lo, hi = split(rv, rr, i)
                wall[VOFF + 2 * i * nkc + r, j * L:(j + 1) * L, :] = lo.T.astype(_BF16)
                wall[VOFF + (2 * i + 1) * nkc + r, j * L:(j + 1) * L, :] = hi.T.astype(_BF16)

    for cp in cq:
        cp.wait()

    def b2(r, carry):
        cs = pl.ds(pl.multiple_of(r * CB, CB), CB)
        pq = pq_ref[:, cs]
        rc = 1.0 / (_nn(z_ref[...], pq) + 1e-6)
        r1 = rc.astype(_BF16)
        e1 = rc - r1.astype(_F32)
        r2 = e1.astype(_BF16)
        r3 = (e1 - r2.astype(_F32)).astype(_BF16)
        rx = _nn(e_ref[...], jnp.concatenate([r1, r2, r3], axis=0))
        pr = (pq.astype(_F32) * rx).astype(_BF16)
        acc_ref[:, cs] = (1.0 - g_ref[:, cs]) * _nn(gt_ref[...], pr)
        for e in range(nqc // nb):
            ext_q(r * (nqc // nb) + e)
        return carry
    jax.lax.fori_loop(0, nb, b2, 0)

    cc.start()
    cw.start()

    hpi = H // nkc

    for gi in range(2):
        for cp in kvcopies(gi):
            cp.wait()

        def qall(rr, carry, gi=gi):
            for t in range(hpi):
                hh = (gi * (nkc // 2) + rr) * hpi + t
                wq_h = jnp.concatenate([wall[QOFF + hh * nqc + t2] for t2 in range(nqc)], axis=1)[:, 0:M]
                qt_s[hh] = _nn(wq_h, xt_ref[...]).astype(_BF16)
                if t == 0:
                    ext_kv(gi, rr)
            return carry
        jax.lax.fori_loop(0, nkc // 2, qall, 0)
    cc.wait()
    cw.wait()

    row = jax.lax.broadcasted_iota(jnp.int32, (TQ, TQ), 0)
    col = jax.lax.broadcasted_iota(jnp.int32, (TQ, TQ), 1)
    cmask = row <= col
    nq = S // TQ

    def head(h, carry):
        k_ref[...] = _nn(c_ref[...], jnp.concatenate([jnp.concatenate([wall[KOFF + (h * (D // L) + j) * KB + b] for b in range(KB)], axis=0) for j in range(D // L)], axis=1)).astype(_BF16)

        def scores(i):
            kv = (i + 1) * TQ
            s = _nn(k_ref[0:kv, :], qt_s[h, :, i * TQ:(i + 1) * TQ])
            sd = jnp.where(cmask, s[i * TQ:, :], -1e9)
            return (s[:i * TQ, :] if i > 0 else None), sd

        def smax(so, sd):
            m = jnp.max(sd, axis=0, keepdims=True)
            if so is not None:
                m = jnp.maximum(m, jnp.max(so, axis=0, keepdims=True))
            return m

        def sexp(so, sd, m):
            pd = jnp.exp(sd - m)
            l = jnp.sum(pd, axis=0, keepdims=True)
            if so is not None:
                po = jnp.exp(so - m)
                l = l + jnp.sum(po, axis=0, keepdims=True)
                p = jnp.concatenate([po.astype(_BF16), pd.astype(_BF16)], axis=0)
            else:
                p = pd.astype(_BF16)
            return p, l

        def pv(i, p, l):
            kv = (i + 1) * TQ
            r = g_ref[:, i * TQ:(i + 1) * TQ] / l
            ctx = _nn(vt_ref[:, 0:kv], p) * r
            ctx_ref[:, i * TQ:(i + 1) * TQ] = ctx.astype(_BF16)

        ss = [scores(j) for j in range(nq)]
        vt_ref[...] = _nt(jnp.concatenate([wall[VOFF + h * nkc + t2] for t2 in range(nkc)], axis=1), c_ref[...]).astype(_BF16)
        m = smax(*ss[0])
        for i in range(nq):
            p, l = sexp(*ss[i], m)
            if i + 1 < nq:
                m = smax(*ss[i + 1])
            pv(i, p, l)

        acc_ref[...] += _nn(wot_ref[h], ctx_ref[...])
        return carry
    jax.lax.fori_loop(0, H, head, 0)

    o_ref[...] = acc_ref[...].astype(o_ref.dtype)


@jax.jit
def pallas_gated_mix__compressed_kv_cla__linear_attn_block__prompt_kernel(
    A_x: jax.Array,
    A_c_kv: jax.Array,
    A_w_q: jax.Array,
    A_w_uk: jax.Array,
    A_w_uv: jax.Array,
    A_w_o: jax.Array,
    B_x: jax.Array,
    B_wqkv: jax.Array,
    B_wo: jax.Array,
    gate_w: jax.Array,
):
    B, S, M = A_x.shape
    Sk, Dc = A_c_kv.shape[1], A_c_kv.shape[2]
    H, D = A_w_q.shape[1], A_w_q.shape[2]
    L = _L
    HB = 16
    TQ = L
    CB = 512
    assert B == 1 and S == Sk and D == 2 * L
    MP = -(-M // L) * L

    xt = A_x.reshape(S, M).T
    c = A_c_kv.reshape(Sk, Dc)
    wq = A_w_q.reshape(M * H, D)
    wuk = A_w_uk.reshape(Dc * H, D)
    wuv = A_w_uv.reshape(Dc * H, D)
    wot = jnp.swapaxes(A_w_o, 1, 2)
    gw = gate_w.reshape(1, M)

    ranges = _bd_ranges(M, M // HB)
    kvrows = max(e1 - e0 for _, _, e0, e1 in ranges) + 16
    kern = functools.partial(_kernel, S=S, M=M, D=D, Dc=Dc, H=H, HB=HB, TQ=TQ, CB=CB,
                             scale=float(D) ** -0.5)
    out = pl.pallas_call(
        kern,
        grid=(1,),
        in_specs=[pl.BlockSpec(memory_space=pl.ANY)] * 9,
        out_specs=pl.BlockSpec((M, S), lambda i: (0, 0)),
        out_shape=jax.ShapeDtypeStruct((M, S), xt.dtype),
        scratch_shapes=[
            pltpu.VMEM((M, S), _BF16), pltpu.VMEM((M, 3 * M), _BF16), pltpu.VMEM((M, M), _BF16),
            pltpu.VMEM((1, M), _BF16), pltpu.VMEM((Sk, Dc), _BF16), pltpu.VMEM((H, M, D), _BF16),
            pltpu.VMEM((MP * H, L), _BF16), pltpu.VMEM((MP * H, L), _BF16),
            *[pltpu.VMEM((Dc * H // 2, L), _BF16) for _ in range(8)],
            pltpu.VMEM((H * (MP // L) + H * (D // L) * (Dc // D) + H * (Dc // L), D, L), _BF16),
            pltpu.VMEM((H, D, S), _BF16),
            pltpu.VMEM((M, S), _F32), pltpu.VMEM((1, S), _F32),
            pltpu.VMEM((Sk, D), _BF16), pltpu.VMEM((D, Sk), _BF16), pltpu.VMEM((D, S), _BF16),
            pltpu.VMEM((3 * M + 16, M), _BF16), pltpu.VMEM((M, S), _BF16),
            pltpu.VMEM((len(ranges), kvrows, L), _F32), pltpu.VMEM((len(ranges), kvrows, L), jnp.int32),
            pltpu.VMEM((M, M), _BF16), pltpu.VMEM((M, M), _BF16),
            pltpu.VMEM((HB, M), _BF16), pltpu.VMEM((M, 3 * HB), _BF16),
            pltpu.SemaphoreType.DMA((7,)), pltpu.SemaphoreType.DMA((S // CB,)),
            pltpu.SemaphoreType.DMA((8,)),
        ],
        compiler_params=pltpu.CompilerParams(
            dimension_semantics=("arbitrary",),
            vmem_limit_bytes=115 * 1024 * 1024,
        ),
    )(xt, B_wqkv, B_wo, gw, wot, c, wq, wuk, wuv)
    return out.T.reshape(B, S, M)
```

```python
import functools

import jax
import jax.numpy as jnp
import jax.experimental.pallas as pl
import jax.experimental.pallas.tpu as pltpu

_F32 = jnp.float32
_BF16 = jnp.bfloat16
_L = 128


def _nt(a, b):
    return jax.lax.dot_general(a, b, (((1,), (1,)), ((), ())), preferred_element_type=_F32)


def _nn(a, b):
    return jnp.dot(a, b, preferred_element_type=_F32)


def _bd_ranges(M, Dh):
    out = []
    for d0 in range(0, M, _L):
        d1 = min(d0 + _L, M)
        e0 = (d0 // Dh) * Dh
        e1 = ((d1 - 1) // Dh + 1) * Dh
        out.append((d0, d1, (e0 // 16) * 16, min(-(-e1 // 16) * 16, M)))
    return out


def _kernel(xt_hbm, wqkv_hbm, wob_hbm, gw_hbm, wot_hbm, c_hbm, wq_hbm, wuk_hbm, wuv_hbm,
            o_ref,
            xt_ref, wqkv_ref, wob_ref, gw_ref, c_ref, wot_ref,
            rq0, rq1, rka0, rka1, rva0, rva1, rkb0, rkb1, rvb0, rvb1, tmp_ref, wall, qt_s,
            acc_ref, g_ref, k_ref, vt_ref, ctx_ref,
            wqkvt_ref, pq_ref, kvt_ref, msk_ref, kvm_ref, gt_ref, z_ref, e_ref,
            sems, xsems, kvsems,
            *, S, M, D, Dc, H, HB, TQ, CB, scale):
    L = _L
    HP = H // 2
    Dh = M // HB
    nb = S // CB
    nkc = Dc // L
    nqc = -(-M // L)
    KB = Dc // D
    QOFF, KOFF, VOFF = 0, H * nqc, H * nqc + H * (D // L) * KB

    cqkv = pltpu.make_async_copy(wqkv_hbm, wqkv_ref, sems.at[0])
    cgw = pltpu.make_async_copy(gw_hbm, gw_ref, sems.at[1])
    cwob = pltpu.make_async_copy(wob_hbm, wob_ref, sems.at[2])
    cq = [
        pltpu.make_async_copy(wq_hbm.at[:, 0:L], rq0.at[0:M * H, :], sems.at[3]),
        pltpu.make_async_copy(wq_hbm.at[:, L:2 * L], rq1.at[0:M * H, :], sems.at[4]),
    ]
    cc = pltpu.make_async_copy(c_hbm, c_ref, sems.at[5])
    cw = pltpu.make_async_copy(wot_hbm, wot_ref, sems.at[6])

    def xcopy(r):
        cs = pl.ds(pl.multiple_of(r * CB, CB), CB)
        return pltpu.make_async_copy(xt_hbm.at[:, cs], xt_ref.at[:, cs], xsems.at[r])

    GR = (Dc // 2) * H
    kvraw = ((rka0, rka1, rva0, rva1), (rkb0, rkb1, rvb0, rvb1))

    def kvcopies(gi):
        rs = pl.ds(gi * GR, GR)
        k0, k1, v0, v1 = kvraw[gi]
        return [
            pltpu.make_async_copy(wuk_hbm.at[rs, 0:L], k0, kvsems.at[4 * gi]),
            pltpu.make_async_copy(wuk_hbm.at[rs, L:2 * L], k1, kvsems.at[4 * gi + 1]),
            pltpu.make_async_copy(wuv_hbm.at[rs, 0:L], v0, kvsems.at[4 * gi + 2]),
            pltpu.make_async_copy(wuv_hbm.at[rs, L:2 * L], v1, kvsems.at[4 * gi + 3]),
        ]

    cqkv.start()
    cgw.start()
    for r in range(nb):
        xcopy(r).start()
    cwob.start()

    rq0[M * H:, :] = jnp.zeros((rq0.shape[0] - M * H, L), _BF16)
    rq1[M * H:, :] = jnp.zeros((rq1.shape[0] - M * H, L), _BF16)
    kvt_ref[...] = jnp.zeros_like(kvt_ref)
    kvm_ref[...] = jnp.zeros_like(kvm_ref)
    ranges = _bd_ranges(M, Dh)
    for t, (d0, d1, e0, e1) in enumerate(ranges):
        he = (jax.lax.broadcasted_iota(jnp.int32, (e1 - e0, d1 - d0), 0) + e0) // Dh
        hd = (jax.lax.broadcasted_iota(jnp.int32, (e1 - e0, d1 - d0), 1) + d0) // Dh
        msk_ref[t, 0:e1 - e0, 0:d1 - d0] = jnp.where(he == hd, 1, 0)
        zr = jax.lax.broadcasted_iota(jnp.int32, (HB, d1 - d0), 0)
        zd = (jax.lax.broadcasted_iota(jnp.int32, (HB, d1 - d0), 1) + d0) // Dh
        msk_ref[t, e1 - e0:e1 - e0 + HB, 0:d1 - d0] = jnp.where(zr == zd, 1, 0)
    er = jax.lax.broadcasted_iota(jnp.int32, (M, 3 * HB), 0) // Dh
    ec = jax.lax.broadcasted_iota(jnp.int32, (M, 3 * HB), 1) % HB
    e_ref[...] = jnp.where(er == ec, 1.0, 0.0).astype(_BF16)

    cqkv.wait()
    cgw.wait()
    for cp in cq:
        cp.start()
    wqkvt_ref[0:3 * M, :] = wqkv_ref[...].T
    wqkvt_ref[3 * M:3 * M + 16, :] = jnp.broadcast_to(gw_ref[...], (16, M))

    def b1(r, carry):
        cs = pl.ds(pl.multiple_of(r * CB, CB), CB)
        xcopy(r).wait()
        for gi in range(2):
            @pl.when(r == gi * (nb // 2))
            def _():
                for cp in kvcopies(gi):
                    cp.start()
        qkvt = _nn(wqkvt_ref[...], xt_ref[:, cs])
        g_ref[:, cs] = jax.nn.sigmoid(qkvt[3 * M:3 * M + 1, :])
        qk = qkvt[0:2 * M, :]
        pqk = (jnp.where(qk > 0, qk + 1.0, jnp.exp(qk)) + 1e-6).astype(_BF16)
        pq_ref[:, cs] = pqk[0:M, :]
        vt = qkvt[2 * M:3 * M, :].astype(_BF16)
        ones = jnp.ones((16, CB), _BF16)
        for t, (d0, d1, e0, e1) in enumerate(ranges):
            v_ext = jnp.concatenate([vt[e0:e1, :], ones], axis=0)
            kvt_ref[t, 0:e1 - e0 + 16, 0:d1 - d0] += _nt(v_ext, pqk[M + d0:M + d1, :])
        return carry
    jax.lax.fori_loop(0, nb, b1, 0)

    for t, (d0, d1, e0, e1) in enumerate(ranges):
        n = e1 - e0
        kz = jnp.where(msk_ref[t, 0:n + HB, 0:d1 - d0] != 0, kvt_ref[t, 0:n + HB, 0:d1 - d0], 0.0).astype(_BF16)
        kvm_ref[e0:e1, d0:d1] = kz[0:n, :]
        z_ref[:, d0:d1] = kz[n:n + HB, :]
    cwob.wait()
    gt_ref[...] = _nn(wob_ref[...].T, kvm_ref[...]).astype(_BF16)

    def stage(raw, r, t):
        rows = raw[pl.ds(pl.multiple_of(r * (L * H), L * H), L * H), :]
        tmp_ref[t] = pltpu.bitcast(rows, jnp.uint32)

    def split(t, i):
        u = tmp_ref[t, pl.ds(i, L, stride=HP), :]
        lo = pltpu.bitcast(u << 16, _F32)
        hi = pltpu.bitcast(u & jnp.uint32(0xFFFF0000), _F32)
        return lo, hi

    def ext_q(r):
        for j, rq in enumerate((rq0, rq1)):
            stage(rq, r, j)
        for i in range(HP):
            for j in range(2):
                lo, hi = split(j, i)
                wall[QOFF + 2 * i * nqc + r, j * L:(j + 1) * L, :] = (lo * scale).T.astype(_BF16)
                wall[QOFF + (2 * i + 1) * nqc + r, j * L:(j + 1) * L, :] = (hi * scale).T.astype(_BF16)

    def ext_kv(gi, rr):
        r = gi * (nkc // 2) + rr
        kb = r // (D // L)
        ks = pl.ds(pl.multiple_of((r % (D // L)) * L, L), L)
        for t, raw in enumerate(kvraw[gi]):
            stage(raw, rr, t)
        for i in range(HP):
            for j in range(2):
                lo, hi = split(j, i)
                wall[KOFF + ((2 * i) * (D // L) + j) * KB + kb, ks, :] = lo.astype(_BF16)
                wall[KOFF + ((2 * i + 1) * (D // L) + j) * KB + kb, ks, :] = hi.astype(_BF16)
                lo, hi = split(2 + j, i)
                wall[VOFF + 2 * i * nkc + r, j * L:(j + 1) * L, :] = lo.T.astype(_BF16)
                wall[VOFF + (2 * i + 1) * nkc + r, j * L:(j + 1) * L, :] = hi.T.astype(_BF16)

    for cp in cq:
        cp.wait()

    def b2(r, carry):
        cs = pl.ds(pl.multiple_of(r * CB, CB), CB)
        pq = pq_ref[:, cs]
        rc = 1.0 / (_nn(z_ref[...], pq) + 1e-6)
        r1 = rc.astype(_BF16)
        e1 = rc - r1.astype(_F32)
        r2 = e1.astype(_BF16)
        r3 = (e1 - r2.astype(_F32)).astype(_BF16)
        rx = _nn(e_ref[...], jnp.concatenate([r1, r2, r3], axis=0))
        pr = (pq.astype(_F32) * rx).astype(_BF16)
        acc_ref[:, cs] = (1.0 - g_ref[:, cs]) * _nn(gt_ref[...], pr)
        for e in range(nqc // nb):
            ext_q(r * (nqc // nb) + e)
        return carry
    jax.lax.fori_loop(0, nb, b2, 0)

    cc.start()
    cw.start()

    hpi = H // nkc

    for gi in range(2):
        for cp in kvcopies(gi):
            cp.wait()

        def qall(rr, carry, gi=gi):
            for t in range(hpi):
                hh = (gi * (nkc // 2) + rr) * hpi + t
                wq_h = jnp.concatenate([wall[QOFF + hh * nqc + t2] for t2 in range(nqc)], axis=1)[:, 0:M]
                qt_s[hh] = _nn(wq_h, xt_ref[...]).astype(_BF16)
                if t == 0:
                    ext_kv(gi, rr)
            return carry
        jax.lax.fori_loop(0, nkc // 2, qall, 0)
    cc.wait()
    cw.wait()

    row = jax.lax.broadcasted_iota(jnp.int32, (TQ, TQ), 0)
    col = jax.lax.broadcasted_iota(jnp.int32, (TQ, TQ), 1)
    cmask = row <= col
    nq = S // TQ

    def head(h, carry):
        k_ref[...] = _nn(c_ref[...], jnp.concatenate([jnp.concatenate([wall[KOFF + (h * (D // L) + j) * KB + b] for b in range(KB)], axis=0) for j in range(D // L)], axis=1)).astype(_BF16)

        def scores(i):
            kv = (i + 1) * TQ
            s = _nn(k_ref[0:kv, :], qt_s[h, :, i * TQ:(i + 1) * TQ])
            sd = jnp.where(cmask, s[i * TQ:, :], -1e9)
            return (s[:i * TQ, :] if i > 0 else None), sd

        def smax(so, sd):
            m = jnp.max(sd, axis=0, keepdims=True)
            if so is not None:
                m = jnp.maximum(m, jnp.max(so, axis=0, keepdims=True))
            return m

        def sexp(so, sd, m):
            pd = jnp.exp(sd - m)
            l = jnp.sum(pd, axis=0, keepdims=True)
            if so is not None:
                po = jnp.exp(so - m)
                l = l + jnp.sum(po, axis=0, keepdims=True)
                p = jnp.concatenate([po.astype(_BF16), pd.astype(_BF16)], axis=0)
            else:
                p = pd.astype(_BF16)
            return p, l

        def pv(i, p, l):
            kv = (i + 1) * TQ
            r = g_ref[:, i * TQ:(i + 1) * TQ] / l
            ctx = _nn(vt_ref[:, 0:kv], p) * r
            ctx_ref[:, i * TQ:(i + 1) * TQ] = ctx.astype(_BF16)

        ss = [scores(j) for j in range(nq)]
        vt_ref[...] = _nt(jnp.concatenate([wall[VOFF + h * nkc + t2] for t2 in range(nkc)], axis=1), c_ref[...]).astype(_BF16)
        m = smax(*ss[0])
        for i in range(nq):
            p, l = sexp(*ss[i], m)
            if i + 1 < nq:
                m = smax(*ss[i + 1])
            pv(i, p, l)

        acc_ref[...] += _nn(wot_ref[h], ctx_ref[...])
        return carry
    jax.lax.fori_loop(0, H, head, 0)

    o_ref[...] = acc_ref[...].astype(o_ref.dtype)


@jax.jit
def pallas_gated_mix__compressed_kv_cla__linear_attn_block__prompt_kernel(
    A_x: jax.Array,
    A_c_kv: jax.Array,
    A_w_q: jax.Array,
    A_w_uk: jax.Array,
    A_w_uv: jax.Array,
    A_w_o: jax.Array,
    B_x: jax.Array,
    B_wqkv: jax.Array,
    B_wo: jax.Array,
    gate_w: jax.Array,
):
    B, S, M = A_x.shape
    Sk, Dc = A_c_kv.shape[1], A_c_kv.shape[2]
    H, D = A_w_q.shape[1], A_w_q.shape[2]
    L = _L
    HB = 16
    TQ = L
    CB = 512
    assert B == 1 and S == Sk and D == 2 * L
    MP = -(-M // L) * L

    xt = A_x.reshape(S, M).T
    c = A_c_kv.reshape(Sk, Dc)
    wq = A_w_q.reshape(M * H, D)
    wuk = A_w_uk.reshape(Dc * H, D)
    wuv = A_w_uv.reshape(Dc * H, D)
    wot = jnp.swapaxes(A_w_o, 1, 2)
    gw = gate_w.reshape(1, M)

    ranges = _bd_ranges(M, M // HB)
    kvrows = max(e1 - e0 for _, _, e0, e1 in ranges) + 16
    kern = functools.partial(_kernel, S=S, M=M, D=D, Dc=Dc, H=H, HB=HB, TQ=TQ, CB=CB,
                             scale=float(D) ** -0.5)
    out = pl.pallas_call(
        kern,
        grid=(1,),
        in_specs=[pl.BlockSpec(memory_space=pl.ANY)] * 9,
        out_specs=pl.BlockSpec((M, S), lambda i: (0, 0)),
        out_shape=jax.ShapeDtypeStruct((M, S), xt.dtype),
        scratch_shapes=[
            pltpu.VMEM((M, S), _BF16), pltpu.VMEM((M, 3 * M), _BF16), pltpu.VMEM((M, M), _BF16),
            pltpu.VMEM((1, M), _BF16), pltpu.VMEM((Sk, Dc), _BF16), pltpu.VMEM((H, M, D), _BF16),
            pltpu.VMEM((MP * H, L), _BF16), pltpu.VMEM((MP * H, L), _BF16),
            *[pltpu.VMEM((Dc * H // 2, L), _BF16) for _ in range(8)],
            pltpu.VMEM((4, L * H // 2, L), jnp.uint32),
            pltpu.VMEM((H * (MP // L) + H * (D // L) * (Dc // D) + H * (Dc // L), D, L), _BF16),
            pltpu.VMEM((H, D, S), _BF16),
            pltpu.VMEM((M, S), _F32), pltpu.VMEM((1, S), _F32),
            pltpu.VMEM((Sk, D), _BF16), pltpu.VMEM((D, Sk), _BF16), pltpu.VMEM((D, S), _BF16),
            pltpu.VMEM((3 * M + 16, M), _BF16), pltpu.VMEM((M, S), _BF16),
            pltpu.VMEM((len(ranges), kvrows, L), _F32), pltpu.VMEM((len(ranges), kvrows, L), jnp.int32),
            pltpu.VMEM((M, M), _BF16), pltpu.VMEM((M, M), _BF16),
            pltpu.VMEM((HB, M), _BF16), pltpu.VMEM((M, 3 * HB), _BF16),
            pltpu.SemaphoreType.DMA((7,)), pltpu.SemaphoreType.DMA((S // CB,)),
            pltpu.SemaphoreType.DMA((8,)),
        ],
        compiler_params=pltpu.CompilerParams(
            dimension_semantics=("arbitrary",),
            vmem_limit_bytes=115 * 1024 * 1024,
        ),
    )(xt, B_wqkv, B_wo, gw, wot, c, wq, wuk, wuv)
    return out.T.reshape(B, S, M)
```
